```python
import jax
import jax.numpy as jnp

def _softmax(x, axis=-1):
    return jax.nn.softmax(x, axis=axis)

def _gelu(x):
    return jax.nn.gelu(x, approximate=True)

def _silu(x):
    return jax.nn.silu(x)

def _sigmoid(x):
    return jax.nn.sigmoid(x)

def _layernorm(x, axis=-1, eps=1e-05):
    m = jnp.mean(x, axis=axis, keepdims=True)
    v = jnp.var(x, axis=axis, keepdims=True)
    return (x - m) / jnp.sqrt(v + eps)

def _scatter_add(tgt, idx, src, axis=0):
    return tgt.at[idx].add(src)

def _segment_sum(src, seg, n):
    return jax.ops.segment_sum(src, seg, n)

class _Rng:

    def __init__(self, key):
        self._k = key

    def _next(self):
        self._k, sub = jax.random.split(self._k)
        return sub

    def normal(self, shape):
        return jax.random.normal(self._next(), shape, dtype=jnp.bfloat16)

    def randint(self, lo, hi, shape):
        return jax.random.randint(self._next(), shape, lo, hi, dtype=jnp.int32)

    def uniform(self, shape, lo=0.0, hi=1.0):
        return jax.random.uniform(self._next(), shape, jnp.bfloat16, lo, hi)

    def permutation(self, n):
        return jax.random.permutation(self._next(), n)
kernel_name = 'concat_heads__memory_aug_recurrent_mem_tr__ssm_conv_h3__prompt'

def setup_inputs():
    _rng = _Rng(jax.random.key(int.from_bytes(__import__("os").urandom(4), "little")))
    _w = lambda a: (lambda t: t.astype(jnp.bfloat16) if jnp.issubdtype(t.dtype, jnp.floating) else t)(jnp.asarray(a))

    def _A_setup():
        B, S, Dm = (1, 2048, 1024)
        H, Dh = (32, 128)
        M, seg = (8, 32)
        seg = min(seg, S)
        S = S // seg * seg
        return {'x': _w((lambda *s: _rng.normal(s) * 0.05)(B, S, Dm)), 'mem0': _w((lambda *s: _rng.normal(s) * 0.05)(B, M, Dm)), 'Wq': _w((lambda *s: _rng.normal(s) * 0.05)(Dm, H, Dh) * Dm ** (-0.5)), 'Wk': _w((lambda *s: _rng.normal(s) * 0.05)(Dm, H, Dh) * Dm ** (-0.5)), 'Wv': _w((lambda *s: _rng.normal(s) * 0.05)(Dm, H, Dh) * Dm ** (-0.5)), 'Wo': _w((lambda *s: _rng.normal(s) * 0.05)(H, Dh, Dm) * (H * Dh) ** (-0.5)), 'seg_len': seg}
    _A_in = _A_setup()

    def _B_setup():
        B, S, D = (1, 2048, 1024)
        ks = 4
        return {'q': _w((lambda *s: _rng.normal(s) * 0.05)(B, S, D)), 'k': _w((lambda *s: _rng.normal(s) * 0.05)(B, S, D)), 'v': _w((lambda *s: _rng.normal(s) * 0.05)(B, S, D)), 'shift_k': _w((lambda *s: _rng.normal(s) * 0.05)(D, ks) * 0.5), 'ssm_k': _w((lambda *s: _rng.normal(s) * 0.05)(D, S) * (1.0 / S ** 0.5)), 'ssm_D': _w((lambda *s: _rng.normal(s) * 0.05)(D))}
    _B_in = _B_setup()
    return {'A_x': _A_in['x'], 'A_mem0': _A_in['mem0'], 'A_Wq': _A_in['Wq'], 'A_Wk': _A_in['Wk'], 'A_Wv': _A_in['Wv'], 'A_Wo': _A_in['Wo'], 'A_seg_len': _A_in['seg_len'], 'B_q': _B_in['q'], 'B_k': _B_in['k'], 'B_v': _B_in['v'], 'B_shift_k': _B_in['shift_k'], 'B_ssm_k': _B_in['ssm_k'], 'B_ssm_D': _B_in['ssm_D']}

def reference(A_x, A_mem0, A_Wq, A_Wk, A_Wv, A_Wo, A_seg_len, B_q, B_k, B_v, B_shift_k, B_ssm_k, B_ssm_D):

    def _A_ref(x, mem0, Wq, Wk, Wv, Wo, seg_len):
        B, S, Dm = x.shape
        H, Dh = (Wq.shape[1], Wq.shape[2])
        M = mem0.shape[1]
        scale = Dh ** (-0.5)
        n_seg = S // seg_len
        L = M + seg_len
        idx = jnp.arange(L)
        mask = (idx[:, None] < M) | (idx[:, None] >= idx[None, :])
        mem = mem0
        outs = []
        for s in range(n_seg):
            xs = x[:, s * seg_len:(s + 1) * seg_len, :].copy()
            h = jnp.concatenate([mem, xs], axis=1)
            q = jnp.einsum('btd,dhe->bhte', h, Wq)
            k = jnp.einsum('btd,dhe->bhte', h, Wk)
            v = jnp.einsum('btd,dhe->bhte', h, Wv)
            scores = jnp.einsum('bhqe,bhke->bhqk', q, k) * scale
            scores = jnp.where(mask[None, None], scores, -1000000000.0)
            p = _softmax(scores, axis=-1)
            o = jnp.einsum('bhqk,bhke->bhqe', p, v)
            o = jnp.einsum('bhte,hed->btd', o, Wo)
            mem = o[:, :M, :].copy()
            outs.append(o[:, M:, :])
        return jnp.concatenate(outs, axis=1)

    def _B_ref(q, k, v, shift_k, ssm_k, ssm_D):
        B, S, D = q.shape
        ks = shift_k.shape[-1]
        k_pad = jnp.pad(k, ((0, 0), (ks - 1, 0), (0, 0)))
        k_shift = jnp.zeros_like(k)
        for t in range(ks):
            k_shift = k_shift + k_pad[:, t:t + S, :] * shift_k[:, ks - 1 - t][None, None, :]
        kv = k_shift * v
        L = 2 * S
        kv_pad = jnp.pad(kv, ((0, 0), (0, S), (0, 0)))
        kf_pad = jnp.pad(ssm_k, ((0, 0), (0, S)))
        kv_f = (lambda x, axes=(-2, -1): jnp.fft.rfft2(x.astype(jnp.float32), axes=axes))(kv_pad[:, None, :, :], axes=(1, 2))
        kf_f = (lambda x, axes=(-2, -1): jnp.fft.rfft2(x.astype(jnp.float32), axes=axes))(kf_pad[:, None, :], axes=(1, 2))
        kf_f = (lambda x, *d: x.transpose(*d))(kf_f, 1, 2, 0)
        y_f = kv_f * kf_f[None, :, :, :]
        y = (lambda x, s, axes=(-2, -1): jnp.fft.irfft2(x, s=s, axes=axes).astype(jnp.bfloat16))(y_f, (1, L), axes=(1, 2))[:, 0, :S, :]
        y = y + kv * ssm_D[None, None, :]
        return q * y
    a = _A_ref(A_x, A_mem0, A_Wq, A_Wk, A_Wv, A_Wo, A_seg_len)
    b = _B_ref(B_q, B_k, B_v, B_shift_k, B_ssm_k, B_ssm_D)
    return jnp.concatenate([a, b], axis=-1)
```

```python
import jax, jax.numpy as jnp, numpy as np
from jax import lax
from jax.experimental import pallas as pl
from jax.experimental.pallas import tpu as pltpu

S=2048; D=1024; NC=16; NT=8; NSEG=64
bf16=jnp.bfloat16; f32=jnp.float32; u32=jnp.uint32

def _consts():
    k = np.arange(128)[:,None]; t = np.arange(128)[None,:]
    th = np.pi*(2*k+1)*t/256.0
    F = np.concatenate([np.cos(th), -np.sin(th)], axis=0)
    G = np.concatenate([np.cos(th).T, -np.sin(th).T], axis=1)/128.0
    return F.astype(np.float32), G.astype(np.float32)

def bf(x): return pltpu.bitcast(x, bf16)

def kernel(x_hbm, mem_ref, wq_hbm, wk_hbm, wv_hbm, wo_hbm,
           q_hbm, k_hbm, v_hbm, skT_ref, h_hbm, d_ref, F_ref, G_ref,
           out_hbm,
           xb, wall, wo, stg, aout, membuf, obuf, sems, wsems, osem):
    def w_copy(mu):
        src = (wq_hbm, wk_hbm, wv_hbm)[mu]
        return pltpu.make_async_copy(src, stg.at[mu].bitcast(bf16), wsems.at[mu])
    def wo_copy(n):
        return pltpu.make_async_copy(wo_hbm.at[:, pl.ds(n*128,128)], wo.at[n], wsems.at[3])
    x_copy = pltpu.make_async_copy(x_hbm, xb, wsems.at[4])

    def b_phase(kb, vb, qb, hb, kvb, Xh, Hh, Zb, ob):
        def in_copies(j):
            cs = pl.ds(j*128, 128)
            return [pltpu.make_async_copy(k_hbm.at[:, cs], kb.at[j], sems.at[0, j]),
                    pltpu.make_async_copy(v_hbm.at[:, cs], vb.at[j], sems.at[1, j]),
                    pltpu.make_async_copy(h_hbm.at[cs, :], hb.at[j], sems.at[2, j]),
                    pltpu.make_async_copy(q_hbm.at[:, cs], qb.at[j], sems.at[3, j])]
        for j in range(NT):
            for c in in_copies(j): c.start()
        for mu in range(3): w_copy(mu).start()
        x_copy.start()
        for n in range(8): wo_copy(n).start()

        sgn = jnp.where(lax.broadcasted_iota(jnp.int32,(8,128),0) % 2 == 0, 1.0, -1.0).astype(f32)
        def tile(j, carry):
            for c in in_copies(j): c.wait()
            l0 = pl.multiple_of(j*128, 128)
            w = skT_ref[:, pl.ds(l0,128)].astype(f32)
            F = F_ref[...]
            for c in range(NC):
                if c == 0:
                    ext = jnp.concatenate([jnp.zeros((8,128), f32), kb[j, 0:128, :].astype(f32)], axis=0)
                else:
                    ext = jnp.concatenate([kb[j, c*128-16:c*128, :].astype(f32)[8:16], kb[j, c*128:(c+1)*128, :].astype(f32)], axis=0)
                ks = ext[8:136]*w[0:1] + ext[7:135]*w[1:2] + ext[6:134]*w[2:3] + ext[5:133]*w[3:4]
                kv = (ks * vb[j, c*128:(c+1)*128, :].astype(f32)).astype(bf16)
                kvb[c*128:(c+1)*128, :] = kv
                Xh[c] = jnp.dot(F, kv, preferred_element_type=f32)
                Hh[c] = lax.dot_general(F, hb[j, :, c*128:(c+1)*128], (((1,),(1,)),((),())), preferred_element_type=f32)
            def grp(g, cc):
                r0 = pl.multiple_of(g*8, 8); r1 = pl.multiple_of(g*8+128, 8)
                def X(c): return Xh[c, pl.ds(r0,8), :], Xh[c, pl.ds(r1,8), :]
                def H(m): return Hh[m, pl.ds(r0,8), :], Hh[m, pl.ds(r1,8), :]
                prev = None
                for b in range(4):
                    acc = [None]*4
                    for m in range(4*b+4):
                        hr, hi = H(m)
                        for i in range(4):
                            c = 4*b+i
                            if m > c: continue
                            xr, xi = X(c-m)
                            pr = xr*hr - xi*hi; pi = xr*hi + xi*hr
                            acc[i] = (pr, pi) if acc[i] is None else (acc[i][0]+pr, acc[i][1]+pi)
                    for i in range(4):
                        c = 4*b+i
                        yr, yi = acc[i]
                        if prev is None: zr, zi = yr, yi
                        else: zr, zi = yr - sgn*prev[1], yi + sgn*prev[0]
                        Zb[c, pl.ds(r0,8), :] = zr; Zb[c, pl.ds(r1,8), :] = zi
                        prev = (yr, yi)
                return cc
            lax.fori_loop(0, 16, grp, 0)
            G = G_ref[...]
            dd = d_ref[:, pl.ds(l0,128)].astype(f32)
            for c in range(NC):
                y = jnp.dot(G, Zb[c].astype(bf16), preferred_element_type=f32)
                rs = slice(c*128,(c+1)*128)
                o = qb[j, rs, :].astype(f32) * (y + kvb[rs,:].astype(f32)*dd)
                ob[j, rs, :] = o.astype(bf16)
            pltpu.make_async_copy(ob.at[j], out_hbm.at[:, pl.ds(D + l0,128)], osem.at[j]).start()
            return carry
        lax.fori_loop(0, NT, tile, 0)
        for j in range(NT):
            pltpu.make_async_copy(ob.at[j], out_hbm.at[:, pl.ds(D + j*128,128)], osem.at[j]).wait()
    pl.run_scoped(b_phase,
        pltpu.VMEM((NT,S,128),bf16), pltpu.VMEM((NT,S,128),bf16), pltpu.VMEM((NT,S,128),bf16),
        pltpu.VMEM((NT,128,S),bf16), pltpu.VMEM((S,128),bf16),
        pltpu.VMEM((NC,256,128),f32), pltpu.VMEM((NC,256,128),f32), pltpu.VMEM((NC,256,128),f32),
        pltpu.VMEM((NT,S,128),bf16))

    def a_phase(pre, xB):
        x_copy.wait()
        for s2 in range(NSEG//2):
            a = xb[64*s2+24:64*s2+32, :]
            b = xb[64*s2+56:64*s2+64, :]
            xB[pl.ds(16*s2, 16), :] = jnp.concatenate([a, b], axis=0)
        def repack(mu, j):
            su = stg.at[mu]
            for i in range(64):
                E = su[pl.ds(256*i + j, 8, stride=32), :]
                O = su[pl.ds(256*i + 16 + j, 8, stride=32), :]
                h0 = (E & 0xffff) | (O << 16)
                h1 = (E >> 16) | (O & jnp.uint32(0xffff0000))
                c0 = pl.multiple_of(j*256, 256)
                wall[mu, pl.ds(8*i, 8), pl.ds(c0, 128)] = h0
                wall[mu, pl.ds(8*i, 8), pl.ds(c0+128, 128)] = h1
        for mu in range(3):
            w_copy(mu).wait()
            def rp(j, c, mu=mu):
                repack(mu, j); return c
            lax.fori_loop(0, 16, rp, 0)
            def pm(g, c, mu=mu):
                cs = pl.ds(pl.multiple_of(g*512, 512), 512)
                pre[mu, :, cs] = jnp.dot(xB[...], bf(wall[mu, :, cs]), preferred_element_type=f32)
                return c
            lax.fori_loop(0, 8, pm, 0)
        for n in range(8): wo_copy(n).wait()

        membuf[...] = mem_ref[...].astype(f32)
        ri = lax.broadcasted_iota(jnp.int32, (40, 40), 0)
        ci = lax.broadcasted_iota(jnp.int32, (40, 40), 1)
        mask = (ri < 8) | (ri >= ci)
        scale = 128 ** -0.5
        wou = wo.bitcast(u32)
        def step(s, carry):
            r0 = pl.multiple_of(s * 32, 32)
            p0 = pl.multiple_of(s * 8, 8)
            xs = xb[pl.ds(r0, 32), :].astype(f32)
            h = jnp.concatenate([membuf[...], xs[0:24]], axis=0)
            def proj(mu, g):
                cs = slice(g * 512, (g + 1) * 512)
                r = jnp.dot(h, bf(wall[mu, :, cs]), preferred_element_type=f32)
                return jnp.concatenate([r, pre[mu, pl.ds(p0, 8), cs]], axis=0)
            def scores(q, k):
                return [lax.dot_general(q[:, j*128:(j+1)*128], k[:, j*128:(j+1)*128], (((1,), (1,)), ((), ())), preferred_element_type=f32) for j in range(4)]
            def softmax(scs):
                ps = []
                for sc in scs:
                    sc = jnp.where(mask, sc * scale, -1e9)
                    m = jnp.max(sc, axis=-1, keepdims=True)
                    p = jnp.exp(sc - m)
                    l = jnp.sum(p, axis=-1, keepdims=True)
                    ps.append(p * (1.0 / l))
                return ps
            def pv(ps, v, g):
                for j in range(4):
                    o = jnp.dot(ps[j], v[:, j*128:(j+1)*128], preferred_element_type=f32)
                    obuf[:, (g * 4 + j) * 128:(g * 4 + j + 1) * 128] = o
            q = proj(0, 0); k = proj(1, 0); v = proj(2, 0)
            for g in range(8):
                sc = scores(q, k)
                if g + 1 < 8:
                    q = proj(0, g + 1); k = proj(1, g + 1)
                    ps = softmax(sc)
                    pv(ps, v, g)
                    v = proj(2, g + 1)
                else:
                    ps = softmax(sc)
                    pv(ps, v, g)
            o_all = obuf[...]
            outs = [jnp.dot(o_all, bf(wou[n]), preferred_element_type=f32) for n in range(8)]
            out = jnp.concatenate(outs, axis=1)
            outb = out.astype(bf16)
            membuf[...] = outb[0:8].astype(f32)
            aout[pl.ds(r0, 32), :] = outb[8:40]
            pltpu.make_async_copy(aout.at[pl.ds(r0, 32), :], out_hbm.at[pl.ds(r0, 32), pl.ds(0, D)], osem.at[NT]).start()
            return carry
        lax.fori_loop(0, NSEG, step, 0)
        pltpu.make_async_copy(aout, out_hbm.at[:, pl.ds(0, D)], osem.at[NT]).wait()
    pl.run_scoped(a_phase, pltpu.VMEM((3, 512, 4096), f32), pltpu.VMEM((512, D), bf16))

@jax.jit
def pallas_concat_heads__memory_aug_recurrent_mem_tr__ssm_conv_h3__prompt_kernel(A_x, A_mem0, A_Wq, A_Wk, A_Wv, A_Wo, A_seg_len, B_q, B_k, B_v, B_shift_k, B_ssm_k, B_ssm_D):
    F,G = _consts()
    any_ = pl.BlockSpec(memory_space=pl.ANY)
    vm = pl.BlockSpec(memory_space=pltpu.VMEM)
    out = pl.pallas_call(kernel, out_shape=jax.ShapeDtypeStruct((S,2*D), bf16),
        in_specs=[any_, vm, any_, any_, any_, any_, any_, any_, any_, vm, any_, vm, vm, vm], out_specs=any_,
        scratch_shapes=[pltpu.VMEM((S,D),bf16), pltpu.VMEM((3,512,4096),u32), pltpu.VMEM((8,4096,128),bf16),
            pltpu.VMEM((3,16384,128),u32), pltpu.VMEM((S,D),bf16), pltpu.VMEM((8,D),f32), pltpu.VMEM((40,4096),f32),
            pltpu.SemaphoreType.DMA((4,NT)), pltpu.SemaphoreType.DMA((5,)), pltpu.SemaphoreType.DMA((NT+1,))],
        compiler_params=pltpu.CompilerParams(vmem_limit_bytes=120*1024*1024), name="kf",
    )(A_x.reshape(S,D), A_mem0.reshape(8,D), A_Wq.reshape(32768,128), A_Wk.reshape(32768,128), A_Wv.reshape(32768,128),
      A_Wo.reshape(4096,D), B_q.reshape(S,D), B_k.reshape(S,D), B_v.reshape(S,D), B_shift_k.T, B_ssm_k, B_ssm_D.reshape(1,D),
      jnp.asarray(F).astype(bf16), jnp.asarray(G).astype(bf16))
    return out.reshape(1,S,2*D)
```

```python
E=lambda k,d: d
import jax, jax.numpy as jnp, numpy as np
from jax import lax
from jax.experimental import pallas as pl
from jax.experimental.pallas import tpu as pltpu

S=2048; D=1024; NC=16; NT=8; NSEG=64
bf16=jnp.bfloat16; f32=jnp.float32; u32=jnp.uint32

def _consts():
    k = np.arange(128)[:,None]; t = np.arange(128)[None,:]
    th = np.pi*(2*k+1)*t/256.0
    F = np.concatenate([np.cos(th), -np.sin(th)], axis=0)
    G = np.concatenate([np.cos(th).T, -np.sin(th).T], axis=1)/128.0
    return F.astype(np.float32), G.astype(np.float32)

def bf(x): return pltpu.bitcast(x, bf16)
NT_ = (((1,),(1,)),((),()))

def kernel(x_hbm, x3_hbm, mem_ref, wq_hbm, wk_hbm, wv_hbm, wo_hbm,
           q_hbm, k_hbm, v_hbm, skT_ref, h_hbm, d_ref, F_ref, G_ref,
           out_hbm,
           xb, xB3, wallE, wallO, wo, stg, aout, membuf, obuf, pbuf, sems, wsems, osem):
    WP = 8
    def w_piece(mu, p):
        src = (wq_hbm, wk_hbm, wv_hbm)[mu]
        R = 32768 // WP
        return pltpu.make_async_copy(src.at[pl.ds(p*R, R), :], stg.at[mu, pl.ds(p*R//2, R//2), :].bitcast(bf16), wsems.at[mu])
    def w_wait(mu):
        src = (wq_hbm, wk_hbm, wv_hbm)[mu]
        pltpu.make_async_copy(src, stg.at[mu].bitcast(bf16), wsems.at[mu]).wait()
    def wo_copy(n):
        return pltpu.make_async_copy(wo_hbm.at[:, pl.ds(n*128,128)], wo.at[n], wsems.at[3])
    x_copy = pltpu.make_async_copy(x_hbm, xb, wsems.at[4])
    xB_copy = pltpu.make_async_copy(x3_hbm.at[:, pl.ds(24, 8), :], xB3, wsems.at[5])

    def b_phase(kb, vb, qb, hb, X0, H0, X1, H1, Z0, Z1, ob, kf0, kf1):
        def kvh_copies(j):
            cs = pl.ds(j*128, 128)
            return [pltpu.make_async_copy(k_hbm.at[:, cs], kb.at[j], sems.at[0, j]),
                    pltpu.make_async_copy(v_hbm.at[:, cs], vb.at[j], sems.at[1, j]),
                    pltpu.make_async_copy(h_hbm.at[cs, :], hb.at[j], sems.at[2, j])]
        def q_copy(j):
            return pltpu.make_async_copy(q_hbm.at[:, pl.ds(j*128, 128)], qb.at[j], sems.at[3, j])
        def o_copy(j):
            return pltpu.make_async_copy(ob.at[j], out_hbm.at[:, pl.ds(D + j*128, 128)], osem.at[j])
        sgn = jnp.where(lax.broadcasted_iota(jnp.int32,(8,128),0) % 2 == 0, 1.0, -1.0).astype(f32)

        def s1_pre(j):
            l0 = j*128
            w = skT_ref[:, pl.ds(l0,128)].astype(f32)
            dd = d_ref[:, pl.ds(l0,128)].astype(f32)
            return [jnp.broadcast_to(w[r:r+1], (8,128)) for r in range(4)], dd
        def s1_c(j, c, w, dd, Xh, Hh, kf):
            F = F_ref[...]
            if E('ROLL',1):
                if c == 0:
                    ext = jnp.concatenate([jnp.zeros((8,128), f32), kb[j, 0:128, :].astype(f32)], axis=0)
                else:
                    ext = jnp.concatenate([kb[j, c*128-16:c*128, :].astype(f32)[8:16], kb[j, c*128:(c+1)*128, :].astype(f32)], axis=0)
                ks = ext[8:136]*w[0][0:1] + ext[7:135]*w[1][0:1] + ext[6:134]*w[2][0:1] + ext[5:133]*w[3][0:1]
                kv = (ks * vb[j, c*128:(c+1)*128, :].astype(f32)).astype(bf16)
            else:
                kf[8+c*128:8+(c+1)*128, :] = kb[j, c*128:(c+1)*128, :].astype(f32)
                kvs = []
                for r in range(16):
                    b = 8 + c*128 + r*8
                    ks = kf[b:b+8, :]*w[0] + kf[b-1:b+7, :]*w[1] + kf[b-2:b+6, :]*w[2] + kf[b-3:b+5, :]*w[3]
                    kvs.append(ks)
                kv = (jnp.concatenate(kvs, axis=0) * vb[j, c*128:(c+1)*128, :].astype(f32)).astype(bf16)
            xh = jnp.dot(F, kv, preferred_element_type=f32)
            hh = lax.dot_general(F, hb[j, :, c*128:(c+1)*128], NT_, preferred_element_type=f32)
            e = hh[0:128]; f = hh[128:256]
            if c == 0: e = e + dd
            Xh[c, 0:256, :] = xh
            if E('M3',1):
                Xh[c, 256:384, :] = xh[0:128] + xh[128:256]
                Hh[c, 0:128, :] = e
                Hh[c, 128:256, :] = f - e
                Hh[c, 256:384, :] = e + f
            else:
                Hh[c, 0:128, :] = e
                Hh[c, 128:256, :] = f
        def s2_g(g, Xh, Hh, Zb):
            r0 = g*8; r1 = g*8+128; r2 = g*8+256
            M3 = E('M3',1); BL = E('BL',4)
            if M3:
                def X(c): return Xh[c, r0:r0+8, :], Xh[c, r1:r1+8, :], Xh[c, r2:r2+8, :]
                def H(m): return Hh[m, r0:r0+8, :], Hh[m, r1:r1+8, :], Hh[m, r2:r2+8, :]
            else:
                def X(c): return Xh[c, r0:r0+8, :], Xh[c, r1:r1+8, :]
                def H(m): return Hh[m, r0:r0+8, :], Hh[m, r1:r1+8, :]
            prev = None
            for b in range(16//BL):
                acc = [None]*BL
                for m in range(BL*b+BL):
                    hm = H(m)
                    for i in range(BL):
                        c = BL*b+i
                        if m > c: continue
                        xc = X(c-m)
                        if M3:
                            he, hfe, hef = hm; xa, xb_, xs_ = xc
                            p = (he*xs_, xa*hfe, xb_*hef)
                        else:
                            hr, hi = hm; xr, xi = xc
                            p = (xr*hr - xi*hi, xr*hi + xi*hr)
                        acc[i] = p if acc[i] is None else tuple(a_+p_ for a_, p_ in zip(acc[i], p))
                for i in range(BL):
                    c = BL*b+i
                    if M3:
                        yr = acc[i][0] - acc[i][2]; yi = acc[i][0] + acc[i][1]
                    else:
                        yr, yi = acc[i]
                    if prev is None: zr, zi = yr, yi
                    else: zr, zi = yr - sgn*prev[1], yi + sgn*prev[0]
                    Zb[c, r0:r0+8, :] = zr; Zb[c, r1:r1+8, :] = zi
                    prev = (yr, yi)
        def s3_c(j, c, Zb):
            G = G_ref[...]
            y = jnp.dot(G, Zb[c].astype(bf16), preferred_element_type=f32)
            rs = slice(c*128,(c+1)*128)
            ob[j, rs, :] = (qb[j, rs, :].astype(f32) * y).astype(bf16)
        def s1(j, Xh, Hh, kf):
            w, dd = s1_pre(j)
            for c in range(NC): s1_c(j, c, w, dd, Xh, Hh, kf)
        def s3(j, Zb):
            for c in range(NC): s3_c(j, c, Zb)
        def fused(j1, XH1, XH0, Zw, j3, Zr):
            if j1 is not None: w, dd = s1_pre(j1)
            for c in range(NC):
                if j1 is not None: s1_c(j1, c, w, dd, *XH1)
                s2_g(c, *XH0, Zw)
                if j3 is not None: s3_c(j3, c, Zr)

        for c in kvh_copies(0): c.start()
        for c in kvh_copies(1): c.start()
        for c in kvh_copies(0): c.wait()
        for c in kvh_copies(2): c.start()
        q_copy(0).start()
        if E('PH',9) >= 2: xB_copy.start()
        kf0[0:8, :] = jnp.zeros((8,128), f32); kf1[0:8, :] = jnp.zeros((8,128), f32)
        s1(0, X0, H0, kf0)
        with jax.named_scope('Bloop'):
          for j in range(NT):
            XHw = (X1, H1, kf1) if j % 2 == 0 else (X0, H0, kf0)
            XHr = (X0, H0) if j % 2 == 0 else (X1, H1)
            Zw, Zr = (Z0, Z1) if j % 2 == 0 else (Z1, Z0)
            if j + 1 < NT:
                for c in kvh_copies(j+1): c.wait()
            if j + 3 < NT:
                for c in kvh_copies(j+3): c.start()
            if j + 1 < NT: q_copy(j+1).start()
            w_piece(0, j).start()
            if j >= 1: q_copy(j-1).wait()
            fused(j+1 if j + 1 < NT else None, XHw, XHr, Zw, j-1 if j >= 1 else None, Zr)
            if j >= 1: o_copy(j-1).start()
        q_copy(NT-1).wait()
        if E('PH',9) >= 3:
            for p in range(WP): w_piece(1, p).start()
        s3(NT-1, Z1)
        o_copy(NT-1).start()
        for j in range(NT): o_copy(j).wait()
    pl.run_scoped(b_phase,
        pltpu.VMEM((NT,S,128),bf16), pltpu.VMEM((NT,S,128),bf16), pltpu.VMEM((NT,S,128),bf16),
        pltpu.VMEM((NT,128,S),bf16),
        *([pltpu.VMEM((NC,384,128),f32)]*4), *([pltpu.VMEM((NC,256,128),f32)]*2),
        pltpu.VMEM((NT,S,128),bf16), pltpu.VMEM((S+8,128),f32), pltpu.VMEM((S+8,128),f32))

    def a_phase(pre, xB):
        xB_copy.wait()
        xB[...] = pltpu.bitcast(xB3[...].reshape(512, D), u32)
        def repack(G, wall):
            mu = G // 8; g = G % 8
            for jj in range(2):
                j = 2*g + jj
                c0 = (g//2)*512 + jj*256
                for i in range(64):
                    Ev = stg[mu, pl.ds(256*i + j, 8, stride=32), :]
                    Ov = stg[mu, pl.ds(256*i + 16 + j, 8, stride=32), :]
                    h0 = (Ev & 0xffff) | (Ov << 16)
                    h1 = (Ev >> 16) | (Ov & jnp.uint32(0xffff0000))
                    wall[mu, pl.ds(8*i, 8), pl.ds(c0, 128)] = h0
                    wall[mu, pl.ds(8*i, 8), pl.ds(c0+128, 128)] = h1
        def pm(G, wall):
            mu = G // 8; g = G % 8
            cs = pl.ds((g//2)*512, 512)
            pre[mu, :, pl.ds(g*512, 512)] = jnp.dot(bf(xB[...]), bf(wall[mu, :, cs]), preferred_element_type=f32)
        w_wait(0)
        repack(0, wallE)
        with jax.named_scope('PRE'):
          for i in range(12):
            if i == 3:
                w_wait(1)
                for p in range(WP): w_piece(2, p).start()
            if i == 7:
                w_wait(2)
                for n in range(8): wo_copy(n).start()
                x_copy.start()
            pm(2*i, wallE)
            repack(2*i+1, wallO)
            pm(2*i+1, wallO)
            if i < 11: repack(2*i+2, wallE)
        for n in range(8): wo_copy(n).wait()
        x_copy.wait()

        membuf[...] = mem_ref[...].astype(f32)
        ri = lax.broadcasted_iota(jnp.int32, (40, 40), 0)
        ci = lax.broadcasted_iota(jnp.int32, (40, 40), 1)
        mask = (ri < 8) | (ri >= ci)
        scale = 128 ** -0.5
        wou = wo.bitcast(u32)
        def step(s, mem):
            r0 = pl.multiple_of(s * 32, 32)
            p0 = pl.multiple_of(s * 8, 8)
            xs = xb[pl.ds(r0, 32), :].astype(f32)
            h = jnp.concatenate([mem, xs[0:24]], axis=0)
            def proj(mu, g):
                wall = wallE if g % 2 == 0 else wallO
                cs = slice((g//2) * 512, (g//2 + 1) * 512)
                r = jnp.dot(h, bf(wall[mu, :, cs]), preferred_element_type=f32)
                return jnp.concatenate([r, pre[mu, pl.ds(p0, 8), g*512:(g+1)*512]], axis=0)
            def scores(q, k):
                return [lax.dot_general(q[:, j*128:(j+1)*128], k[:, j*128:(j+1)*128], NT_, preferred_element_type=f32) for j in range(4)]
            def softmax(scs):
                ps = []
                for sc in scs:
                    sc = jnp.where(mask, sc * scale, -1e9)
                    m = jnp.max(sc, axis=-1, keepdims=True)
                    p = jnp.exp(sc - m)
                    l = jnp.sum(p, axis=-1, keepdims=True)
                    ps.append(p * (1.0 / l))
                return ps
            def pv(ps, v, g):
                for j in range(4):
                    o = jnp.dot(ps[j], v[:, j*128:(j+1)*128], preferred_element_type=f32)
                    obuf[:, (g * 4 + j) * 128:(g * 4 + j + 1) * 128] = o
            q = proj(0, 0); k = proj(1, 0); v = proj(2, 0)
            ORD = "D"
            def p1dots(ns):
                o1 = obuf[:, 0:3584]
                for n in ns:
                    pbuf[:, n*128:(n+1)*128] = jnp.dot(o1, bf(wou[n, 0:1792, :]), preferred_element_type=f32)
            for g in range(8):
                if g + 1 < 8:
                    if ORD == "A":
                        sc = scores(q, k)
                        q = proj(0, g + 1); k = proj(1, g + 1)
                        ps = softmax(sc)
                        pv(ps, v, g)
                        v = proj(2, g + 1)
                    elif ORD == "C":
                        sc = scores(q, k)
                        q = proj(0, g + 1); k = proj(1, g + 1)
                        ps = softmax(sc)
                        vn = proj(2, g + 1)
                        pv(ps, v, g)
                        v = vn
                    elif ORD == "D":
                        qn = proj(0, g + 1)
                        sc = scores(q, k)
                        kn = proj(1, g + 1)
                        ps = softmax(sc)
                        vn = proj(2, g + 1)
                        pv(ps, v, g)
                        q, k, v = qn, kn, vn
                    elif ORD == "E":
                        qn = proj(0, g + 1)
                        sc = scores(q, k)
                        kn = proj(1, g + 1)
                        vn = proj(2, g + 1)
                        ps = softmax(sc)
                        pv(ps, v, g)
                        q, k, v = qn, kn, vn
                else:
                    if ORD in ("A","C"):
                        sc = scores(q, k)
                        p1dots(range(4))
                        ps = softmax(sc)
                        pv(ps, v, g)
                        p1dots(range(4, 8))
                    else:
                        p1dots(range(2))
                        sc = scores(q, k)
                        p1dots(range(2, 5))
                        ps = softmax(sc)
                        pv(ps, v, g)
                        p1dots(range(5, 8))
            o2 = obuf[:, 3584:4096]
            outs = [pbuf[:, n*128:(n+1)*128] + jnp.dot(o2, bf(wou[n, 1792:2048, :]), preferred_element_type=f32) for n in range(8)]
            out = jnp.concatenate(outs, axis=1)
            outb = out.astype(bf16)
            newmem = outb[0:8].astype(f32)
            aout[pl.ds(r0, 32), :] = outb[8:40]
            pltpu.make_async_copy(aout.at[pl.ds(r0, 32), :], out_hbm.at[pl.ds(r0, 32), pl.ds(0, D)], osem.at[NT]).start()
            return newmem
        UN = E('UN',2)
        def stepn(t, carry):
            mem = membuf[...]
            for u in range(UN):
                mem = step(t*UN+u, mem)
            membuf[...] = mem
            return carry
        if E('PH',9) >= 4:
          with jax.named_scope('chain'):
            lax.fori_loop(0, E('NSEG',64)//UN, stepn, 0)
          pltpu.make_async_copy(aout.at[pl.ds(0,32*E('NSEG',64))], out_hbm.at[pl.ds(0,32*E('NSEG',64)), pl.ds(0, D)], osem.at[NT]).wait()
    if E('PH',9) == 2:
        xB_copy.wait(); w_wait(0)
    if E('PH',9) >= 3: pl.run_scoped(a_phase, pltpu.VMEM((3, 512, 4096), f32), pltpu.VMEM((256, D), u32))

@jax.jit
def pallas_concat_heads__memory_aug_recurrent_mem_tr__ssm_conv_h3__prompt_kernel(A_x, A_mem0, A_Wq, A_Wk, A_Wv, A_Wo, A_seg_len, B_q, B_k, B_v, B_shift_k, B_ssm_k, B_ssm_D):
    F,G = _consts()
    any_ = pl.BlockSpec(memory_space=pl.ANY)
    vm = pl.BlockSpec(memory_space=pltpu.VMEM)
    out = pl.pallas_call(kernel, out_shape=jax.ShapeDtypeStruct((S,2*D), bf16),
        in_specs=[any_, any_, vm, any_, any_, any_, any_, any_, any_, any_, vm, any_, vm, vm, vm], out_specs=any_,
        scratch_shapes=[pltpu.VMEM((S,D),bf16), pltpu.VMEM((64,8,D),bf16), pltpu.VMEM((3,512,2048),u32), pltpu.VMEM((3,512,2048),u32),
            pltpu.VMEM((8,4096,128),bf16),
            pltpu.VMEM((3,16384,128),u32), pltpu.VMEM((S,D),bf16), pltpu.VMEM((8,D),f32), pltpu.VMEM((40,4096),f32), pltpu.VMEM((40,1024),f32),
            pltpu.SemaphoreType.DMA((4,NT)), pltpu.SemaphoreType.DMA((6,)), pltpu.SemaphoreType.DMA((NT+1,))],
        compiler_params=pltpu.CompilerParams(vmem_limit_bytes=124*1024*1024), name="kf",
    )(A_x.reshape(S,D), A_x.reshape(64,32,D), A_mem0.reshape(8,D), A_Wq.reshape(32768,128), A_Wk.reshape(32768,128), A_Wv.reshape(32768,128),
      A_Wo.reshape(4096,D), B_q.reshape(S,D), B_k.reshape(S,D), B_v.reshape(S,D), B_shift_k.T, B_ssm_k, B_ssm_D.reshape(1,D),
      jnp.asarray(F).astype(bf16), jnp.asarray(G).astype(bf16))
    return out.reshape(1,S,2*D)
```

```python
import jax, jax.numpy as jnp, numpy as np
from jax import lax
from jax.experimental import pallas as pl
from jax.experimental.pallas import tpu as pltpu

S=2048; D=1024; NC=16; NT=8; NSEG=64
bf16=jnp.bfloat16; f32=jnp.float32; u32=jnp.uint32

def _consts():
    k = np.arange(128)[:,None]; t = np.arange(128)[None,:]
    th = np.pi*(2*k+1)*t/256.0
    F = np.concatenate([np.cos(th), -np.sin(th)], axis=0)
    G = np.concatenate([np.cos(th).T, -np.sin(th).T], axis=1)/128.0
    return F.astype(np.float32), G.astype(np.float32)

def bf(x): return pltpu.bitcast(x, bf16)
NT_ = (((1,),(1,)),((),()))
NSTG = 4

def kernel(zr_ref, x_hbm, x3_hbm, mem_ref, wq_hbm, wk_hbm, wv_hbm, wo_hbm,
           q_hbm, k_hbm, v_hbm, skT_ref, h_hbm, d_ref, F_ref, G_ref,
           out_hbm,
           xb, xB3, xB, wall, wo, stg, aout, membuf, obuf, pbuf, pre,
           kb, vb, qb, hb, ob, X0, H0, X1, H1, Z0, Z1, kf0, kf1,
           sems, wsems, ssems, osem):
    def w_piece(u):
        mu, kk = u // 8, u % 8
        src = (wq_hbm, wk_hbm, wv_hbm)[mu]
        return pltpu.make_async_copy(src.at[pl.ds(kk*4096, 4096), :], stg.at[u % NSTG].bitcast(bf16), ssems.at[u % NSTG])
    def x_piece(p, sem):
        return pltpu.make_async_copy(x_hbm.at[pl.ds(p*256, 256), :], xb.at[pl.ds(p*256, 256), :], wsems.at[sem])
    def wo_copy(n):
        return pltpu.make_async_copy(wo_hbm.at[:, pl.ds(n*128,128)], wo.at[n], wsems.at[0])
    xB_copy = pltpu.make_async_copy(x3_hbm.at[:, pl.ds(24, 8), :], xB3, wsems.at[3])
    def kvh_copies(j):
        cs = pl.ds(j*128, 128); sl = j % 2
        return [pltpu.make_async_copy(k_hbm.at[:, cs], kb.at[sl], sems.at[0, sl]),
                pltpu.make_async_copy(v_hbm.at[:, cs], vb.at[sl], sems.at[1, sl]),
                pltpu.make_async_copy(h_hbm.at[cs, :], hb.at[sl], sems.at[2, sl])]
    def q_copy(j):
        return pltpu.make_async_copy(q_hbm.at[:, pl.ds(j*128, 128)], qb.at[j % 2], sems.at[3, j % 2])
    ob_copy = pltpu.make_async_copy(ob, out_hbm.at[:, pl.ds(D, D)], osem.at[0])
    sgn = jnp.where(lax.broadcasted_iota(jnp.int32,(8,128),0) % 2 == 0, 1.0, -1.0).astype(f32)

    def s1_pre(j):
        l0 = j*128
        w = skT_ref[:, l0:l0+128].astype(f32)
        dd = d_ref[:, l0:l0+128].astype(f32)
        return [jnp.broadcast_to(w[r:r+1], (8,128)) for r in range(4)], dd
    def s1_c(j, c, w, dd):
        Xh, Hh, kf = (X0, H0, kf0) if j % 2 == 0 else (X1, H1, kf1)
        sl = j % 2
        F = F_ref[...]
        kf[8+c*128:8+(c+1)*128, :] = kb[sl, c*128:(c+1)*128, :].astype(f32)
        kvs = []
        for r in range(16):
            b = 8 + c*128 + r*8
            kvs.append(kf[b:b+8, :]*w[0] + kf[b-1:b+7, :]*w[1] + kf[b-2:b+6, :]*w[2] + kf[b-3:b+5, :]*w[3])
        kv = (jnp.concatenate(kvs, axis=0) * vb[sl, c*128:(c+1)*128, :].astype(f32)).astype(bf16)
        xh = jnp.dot(F, kv, preferred_element_type=f32)
        hh = lax.dot_general(F, hb[sl, :, c*128:(c+1)*128], NT_, preferred_element_type=f32)
        e = hh[0:128]; f = hh[128:256]
        if c == 0: e = e + dd
        Xh[c, 0:256, :] = xh
        Xh[c, 256:384, :] = xh[0:128] + xh[128:256]
        Hh[c, 0:128, :] = e
        Hh[c, 128:256, :] = f - e
        Hh[c, 256:384, :] = e + f
    BL = 4
    HK = []
    def s2_gen(j, g):
        Xh, Hh, Zb = (X0, H0, Z0) if j % 2 == 0 else (X1, H1, Z1)
        r0 = g*8; r1 = g*8+128; r2 = g*8+256
        def X(c): return Xh[c, r0:r0+8, :], Xh[c, r1:r1+8, :], Xh[c, r2:r2+8, :]
        def H(m): return Hh[m, r0:r0+8, :], Hh[m, r1:r1+8, :], Hh[m, r2:r2+8, :]
        prev = None
        for b in range(16//BL):
            acc = [None]*BL
            for m in range(BL*b+BL):
                he, hfe, hef = H(m)
                for i in range(BL):
                    c = BL*b+i
                    if m > c: continue
                    xa, xb_, xs_ = X(c-m)
                    p = (he*xs_, xa*hfe, xb_*hef)
                    acc[i] = p if acc[i] is None else tuple(a_+p_ for a_, p_ in zip(acc[i], p))
            for i in range(BL):
                c = BL*b+i
                yr = acc[i][0] - acc[i][2]; yi = acc[i][0] + acc[i][1]
                if prev is None: zr, zi = yr, yi
                else: zr, zi = yr - sgn*prev[1], yi + sgn*prev[0]
                Zb[c, r0:r0+8, :] = zr; Zb[c, r1:r1+8, :] = zi
                prev = (yr, yi)
                HK.append(pltpu.bitcast(zr, u32) | pltpu.bitcast(zi, u32))
            yield None
    def s3_c(j, c):
        Zb = Z0 if j % 2 == 0 else Z1
        G = G_ref[...]
        y = jnp.dot(G, Zb[c].astype(bf16), preferred_element_type=f32)
        rs = slice(c*128,(c+1)*128)
        ob[rs, j*128:(j+1)*128] = (qb[j % 2, rs, :].astype(f32) * y).astype(bf16)

    def repack(u):
        mu, kk = u // 8, u % 8
        sl = u % NSTG
        for i in range(8):
            for j in range(16):
                Ev = stg[sl, pl.ds(256*i + j, 8, stride=32), :]
                Ov = stg[sl, pl.ds(256*i + 16 + j, 8, stride=32), :]
                r0 = kk*64 + 8*i
                wall[mu, r0:r0+8, 256*j:256*j+128] = (Ev & 0xffff) | (Ov << 16)
                wall[mu, r0:r0+8, 256*j+128:256*j+256] = (Ev >> 16) | (Ov & jnp.uint32(0xffff0000))
    def pm_kh(u, g):
        mu, kk = u // 8, u % 8
        pieces = [xB[8*r:8*r+8, 128*kk:128*kk+128] for r in range(32)]
        n = len(HK)
        if n:
            z = zr_ref[...]
            for i, hk in enumerate(HK):
                rg = (i * 32) // n
                pieces[rg] = pieces[rg] | (hk & z)
            HK.clear()
        lhs = jnp.concatenate(pieces, axis=0)
        r = jnp.dot(bf(lhs), bf(wall[mu, kk*64:(kk+1)*64, g*512:(g+1)*512]), preferred_element_type=f32)
        if kk == 0: pre[mu, :, g*512:(g+1)*512] = r
        else: pre[mu, :, g*512:(g+1)*512] += r
    def pm_unit(u, gens):
        steps = [gi for gi in range(len(gens)) for _ in range(16 // BL)]
        n = len(steps)
        for g in range(8):
            for gi in steps[g*n//8:(g+1)*n//8]: next(gens[gi])
            pm_kh(u, g)
    def xb_prep():
        for i in range(NSEG//2):
            ab = jnp.concatenate([xB3[2*i], xB3[2*i+1]], axis=0)
            xB[8*i:8*i+8, :] = pltpu.bitcast(ab, u32)

    xB_copy.start()
    w_piece(0).start()
    kf0[0:8, :] = jnp.zeros((8,128), f32); kf1[0:8, :] = jnp.zeros((8,128), f32)
    xB_copy.wait()
    for c in kvh_copies(0): c.start()
    w_piece(1).start()
    with jax.named_scope('ph1'):
        xb_prep()
        w_piece(0).wait()
        w_piece(2).start()
        repack(0)
    rng3 = (range(0,5), range(5,10), range(10,16))
    rng2 = (range(0,8), range(8,16))
    def sched(u):
        if u == 0: return None, False, []
        if u <= 21: return (u-1)//3, (u-1) % 3 == 0, rng3[(u-1) % 3]
        return 7, u == 22, rng2[u-22]
    with jax.named_scope('ph2'):
        for c in kvh_copies(0): c.wait()
        for c in kvh_copies(1): c.start()
        for u in range(24):
            j, first, cs = sched(u)
            pm_unit(u, [s2_gen(j, c) for c in cs])
            if u == 0:
                w, dd = s1_pre(0)
                for c in range(NC): s1_c(0, c, w, dd)
            else:
                if j + 1 < NT: w, dd = s1_pre(j+1)
                for c in cs:
                    if j + 1 < NT: s1_c(j+1, c, w, dd)
                    if j >= 1: s3_c(j-1, c)
            if u < 23:
                w_piece(u+1).wait()
                jn, firstn, _ = sched(u+1)
                if firstn:
                    if jn + 1 < NT:
                        for c in kvh_copies(jn+1): c.wait()
                    if jn >= 1: q_copy(jn-1).wait()
                    if jn + 2 < NT:
                        for c in kvh_copies(jn+2): c.start()
                    q_copy(jn).start()
                if u + 3 < 24: w_piece(u+3).start()
                if 1 <= u < 17 and u % 2 == 1: wo_copy((u-1)//2).start()
                if u == 18: x_piece(0, 1).start()
                repack(u+1)
        q_copy(NT-1).wait()
        for c in range(NC): s3_c(NT-1, c)
        ob_copy.start()
    for n in range(8): wo_copy(n).wait()
    x_piece(0, 1).wait()
    for p in range(1, 8): x_piece(p, 2).start()

    membuf[...] = mem_ref[...].astype(f32)
    ri = lax.broadcasted_iota(jnp.int32, (40, 40), 0)
    ci = lax.broadcasted_iota(jnp.int32, (40, 40), 1)
    mask = (ri < 8) | (ri >= ci)
    scale = 128 ** -0.5
    wou = wo.bitcast(u32)
    def step(s, mem):
        r0 = pl.multiple_of(s * 32, 32)
        p0 = pl.multiple_of(s * 8, 8)
        xs = xb[pl.ds(r0, 32), :].astype(f32)
        h = jnp.concatenate([mem, xs[0:24]], axis=0)
        def proj(mu, g):
            cs = slice(g * 512, (g + 1) * 512)
            r = jnp.dot(h, bf(wall[mu, :, cs]), preferred_element_type=f32)
            return jnp.concatenate([r, pre[mu, pl.ds(p0, 8), cs]], axis=0)
        def scores(q, k):
            return [lax.dot_general(q[:, j*128:(j+1)*128], k[:, j*128:(j+1)*128], NT_, preferred_element_type=f32) for j in range(4)]
        def softmax(scs):
            ps = []
            for sc in scs:
                sc = jnp.where(mask, sc * scale, -1e9)
                m = jnp.max(sc, axis=-1, keepdims=True)
                p = jnp.exp(sc - m)
                l = jnp.sum(p, axis=-1, keepdims=True)
                ps.append(p * (1.0 / l))
            return ps
        def pv(ps, v, g):
            for j in range(4):
                o = jnp.dot(ps[j], v[:, j*128:(j+1)*128], preferred_element_type=f32)
                obuf[:, (g * 4 + j) * 128:(g * 4 + j + 1) * 128] = o
        def p1dots(ns):
            o1 = obuf[:, 0:3584]
            for n in ns:
                pbuf[:, n*128:(n+1)*128] = jnp.dot(o1, bf(wou[n, 0:1792, :]), preferred_element_type=f32)
        q = proj(0, 0); k = proj(1, 0); v = proj(2, 0)
        for g in range(8):
            if g + 1 < 8:
                qn = proj(0, g + 1)
                sc = scores(q, k)
                kn = proj(1, g + 1)
                ps = softmax(sc)
                vn = proj(2, g + 1)
                pv(ps, v, g)
                q, k, v = qn, kn, vn
            else:
                p1dots(range(2))
                sc = scores(q, k)
                p1dots(range(2, 5))
                ps = softmax(sc)
                pv(ps, v, g)
                p1dots(range(5, 8))
        o2 = obuf[:, 3584:4096]
        outs = [pbuf[:, n*128:(n+1)*128] + jnp.dot(o2, bf(wou[n, 1792:2048, :]), preferred_element_type=f32) for n in range(8)]
        outb = jnp.concatenate(outs, axis=1).astype(bf16)
        newmem = outb[0:8].astype(f32)
        aout[pl.ds(r0, 32), :] = outb[8:40]
        pltpu.make_async_copy(aout.at[pl.ds(r0, 32), :], out_hbm.at[pl.ds(r0, 32), pl.ds(0, D)], osem.at[1]).start()
        return newmem
    UN = 2
    def stepn(t, carry):
        @pl.when(t == (4 // UN) * 2 - 1)
        def _():
            pltpu.make_async_copy(x_hbm.at[pl.ds(256, 7*256), :], xb.at[pl.ds(256, 7*256), :], wsems.at[2]).wait()
        mem = membuf[...]
        for u in range(UN):
            mem = step(t*UN+u, mem)
        membuf[...] = mem
        return carry
    with jax.named_scope('chain'):
        lax.fori_loop(0, NSEG//UN, stepn, 0)
    ob_copy.wait()
    pltpu.make_async_copy(aout, out_hbm.at[:, pl.ds(0, D)], osem.at[1]).wait()

@jax.jit
def pallas_concat_heads__memory_aug_recurrent_mem_tr__ssm_conv_h3__prompt_kernel(A_x, A_mem0, A_Wq, A_Wk, A_Wv, A_Wo, A_seg_len, B_q, B_k, B_v, B_shift_k, B_ssm_k, B_ssm_D):
    F,G = _consts()
    any_ = pl.BlockSpec(memory_space=pl.ANY)
    vm = pl.BlockSpec(memory_space=pltpu.VMEM)
    V = pltpu.VMEM
    out = pl.pallas_call(kernel, out_shape=jax.ShapeDtypeStruct((S,2*D), bf16),
        in_specs=[vm, any_, any_, vm, any_, any_, any_, any_, any_, any_, any_, vm, any_, vm, vm, vm], out_specs=any_,
        scratch_shapes=[V((S,D),bf16), V((64,8,D),bf16), V((256,D),u32), V((3,512,4096),u32),
            V((8,4096,128),bf16), V((NSTG,2048,128),u32), V((S,D),bf16), V((8,D),f32), V((40,4096),f32), V((40,1024),f32),
            V((3,512,4096),f32),
            V((2,S,128),bf16), V((2,S,128),bf16), V((2,S,128),bf16), V((2,128,S),bf16), V((S,D),bf16),
            V((NC,384,128),f32), V((NC,384,128),f32), V((NC,384,128),f32), V((NC,384,128),f32),
            V((NC,256,128),f32), V((NC,256,128),f32), V((S+8,128),f32), V((S+8,128),f32),
            pltpu.SemaphoreType.DMA((4,2)), pltpu.SemaphoreType.DMA((4,)), pltpu.SemaphoreType.DMA((NSTG,)), pltpu.SemaphoreType.DMA((2,))],
        compiler_params=pltpu.CompilerParams(vmem_limit_bytes=124*1024*1024), name="kf",
    )(jnp.asarray(np.zeros((8,128), np.uint32)), A_x.reshape(S,D), A_x.reshape(64,32,D), A_mem0.reshape(8,D), A_Wq.reshape(32768,128), A_Wk.reshape(32768,128), A_Wv.reshape(32768,128),
      A_Wo.reshape(4096,D), B_q.reshape(S,D), B_k.reshape(S,D), B_v.reshape(S,D), B_shift_k.T, B_ssm_k, B_ssm_D.reshape(1,D),
      jnp.asarray(F).astype(bf16), jnp.asarray(G).astype(bf16))
    return out.reshape(1,S,2*D)
```

```python
import jax, jax.numpy as jnp, numpy as np
from jax import lax
from jax.experimental import pallas as pl
from jax.experimental.pallas import tpu as pltpu

S=2048; D=1024; NC=16; NT=8; NSEG=64
bf16=jnp.bfloat16; f32=jnp.float32; u32=jnp.uint32

def _consts():
    k = np.arange(128)[:,None]; t = np.arange(128)[None,:]
    th = np.pi*(2*k+1)*t/256.0
    F = np.concatenate([np.cos(th), -np.sin(th)], axis=0)
    G = np.concatenate([np.cos(th).T, -np.sin(th).T], axis=1)/128.0
    return F.astype(np.float32), G.astype(np.float32)

def bf(x): return pltpu.bitcast(x, bf16)
NT_ = (((1,),(1,)),((),()))
NSTG = 4

def kernel(zr_hbm, x_hbm, x3_hbm, mem_hbm, wq_hbm, wk_hbm, wv_hbm, wo_hbm,
           q_hbm, k_hbm, v_hbm, skT_hbm, h_hbm, d_hbm, F_hbm, G_hbm,
           out_hbm,
           zr_ref, mem_ref, skT_ref, d_ref, F_ref, G_ref, csem,
           xb, xB3, xB, wall, wo, stg, aout, membuf, obuf, pbuf, pre,
           kb, vb, qb, hb, ob, X0, H0, X1, H1, Z0, Z1, kf0, kf1,
           sems, wsems, ssems, osem):
    def w_piece(u):
        mu, kk = u // 8, u % 8
        src = (wq_hbm, wk_hbm, wv_hbm)[mu]
        return pltpu.make_async_copy(src.at[pl.ds(kk*4096, 4096), :], stg.at[u % NSTG].bitcast(bf16), ssems.at[u % NSTG])
    def x_piece(p, sem):
        return pltpu.make_async_copy(x_hbm.at[pl.ds(p*256, 256), :], xb.at[pl.ds(p*256, 256), :], wsems.at[sem])
    def wo_copy(n):
        return pltpu.make_async_copy(wo_hbm.at[:, pl.ds(n*128,128)], wo.at[n], wsems.at[0])
    xB_copy = pltpu.make_async_copy(x3_hbm.at[:, pl.ds(24, 8), :], xB3, wsems.at[3])
    def kvh_copies(j):
        cs = pl.ds(j*128, 128); sl = j % 2
        return [pltpu.make_async_copy(k_hbm.at[:, cs], kb.at[sl], sems.at[0, sl]),
                pltpu.make_async_copy(v_hbm.at[:, cs], vb.at[sl], sems.at[1, sl]),
                pltpu.make_async_copy(h_hbm.at[cs, :], hb.at[sl], sems.at[2, sl])]
    def q_copy(j):
        return pltpu.make_async_copy(q_hbm.at[:, pl.ds(j*128, 128)], qb.at[j % 2], sems.at[3, j % 2])
    ob_copy = pltpu.make_async_copy(ob, out_hbm.at[:, pl.ds(D, D)], osem.at[0])
    sgn = jnp.where(lax.broadcasted_iota(jnp.int32,(8,128),0) % 2 == 0, 1.0, -1.0).astype(f32)

    def s1_pre(j):
        l0 = j*128
        w = skT_ref[:, l0:l0+128].astype(f32)
        dd = d_ref[l0:l0+128].astype(f32).reshape(1, 128)
        return [jnp.broadcast_to(w[r:r+1], (8,128)) for r in range(4)], dd
    def s1_c(j, c, w, dd):
        Xh, Hh, kf = (X0, H0, kf0) if j % 2 == 0 else (X1, H1, kf1)
        sl = j % 2
        F = F_ref[...]
        kf[8+c*128:8+(c+1)*128, :] = kb[sl, c*128:(c+1)*128, :].astype(f32)
        kvs = []
        for r in range(16):
            b = 8 + c*128 + r*8
            kvs.append(kf[b:b+8, :]*w[0] + kf[b-1:b+7, :]*w[1] + kf[b-2:b+6, :]*w[2] + kf[b-3:b+5, :]*w[3])
        kv = (jnp.concatenate(kvs, axis=0) * vb[sl, c*128:(c+1)*128, :].astype(f32)).astype(bf16)
        xh = jnp.dot(F, kv, preferred_element_type=f32)
        hh = lax.dot_general(F, hb[sl, :, c*128:(c+1)*128], NT_, preferred_element_type=f32)
        e = hh[0:128]; f = hh[128:256]
        if c == 0: e = e + dd
        Xh[c, 0:256, :] = xh
        Xh[c, 256:384, :] = xh[0:128] + xh[128:256]
        Hh[c, 0:128, :] = e
        Hh[c, 128:256, :] = f - e
        Hh[c, 256:384, :] = e + f
    BL = 4
    HK = []
    def s2_gen(j, g):
        Xh, Hh, Zb = (X0, H0, Z0) if j % 2 == 0 else (X1, H1, Z1)
        r0 = g*8; r1 = g*8+128; r2 = g*8+256
        def X(c): return Xh[c, r0:r0+8, :], Xh[c, r1:r1+8, :], Xh[c, r2:r2+8, :]
        def H(m): return Hh[m, r0:r0+8, :], Hh[m, r1:r1+8, :], Hh[m, r2:r2+8, :]
        prev = None
        for b in range(16//BL):
            acc = [None]*BL
            for m in range(BL*b+BL):
                he, hfe, hef = H(m)
                for i in range(BL):
                    c = BL*b+i
                    if m > c: continue
                    xa, xb_, xs_ = X(c-m)
                    p = (he*xs_, xa*hfe, xb_*hef)
                    acc[i] = p if acc[i] is None else tuple(a_+p_ for a_, p_ in zip(acc[i], p))
            for i in range(BL):
                c = BL*b+i
                yr = acc[i][0] - acc[i][2]; yi = acc[i][0] + acc[i][1]
                if prev is None: zr, zi = yr, yi
                else: zr, zi = yr - sgn*prev[1], yi + sgn*prev[0]
                Zb[c, r0:r0+8, :] = zr; Zb[c, r1:r1+8, :] = zi
                prev = (yr, yi)
                HK.append(pltpu.bitcast(zr, u32) | pltpu.bitcast(zi, u32))
            yield None
    def s3_c(j, c):
        Zb = Z0 if j % 2 == 0 else Z1
        G = G_ref[...]
        y = jnp.dot(G, Zb[c].astype(bf16), preferred_element_type=f32)
        rs = slice(c*128,(c+1)*128)
        ob[rs, j*128:(j+1)*128] = (qb[j % 2, rs, :].astype(f32) * y).astype(bf16)

    def repack(u):
        mu, kk = u // 8, u % 8
        sl = u % NSTG
        for i in range(8):
            for j in range(16):
                Ev = stg[sl, pl.ds(256*i + j, 8, stride=32), :]
                Ov = stg[sl, pl.ds(256*i + 16 + j, 8, stride=32), :]
                r0 = kk*64 + 8*i
                wall[mu, r0:r0+8, 256*j:256*j+128] = (Ev & 0xffff) | (Ov << 16)
                wall[mu, r0:r0+8, 256*j+128:256*j+256] = (Ev >> 16) | (Ov & jnp.uint32(0xffff0000))
    def pm_kh(u, g):
        mu, kk = u // 8, u % 8
        pieces = [xB[8*r:8*r+8, 128*kk:128*kk+128] for r in range(32)]
        n = len(HK)
        if n:
            z = zr_ref[...]
            for i, hk in enumerate(HK):
                rg = (i * 32) // n
                pieces[rg] = pieces[rg] | (hk & z)
            HK.clear()
        lhs = jnp.concatenate(pieces, axis=0)
        r = jnp.dot(bf(lhs), bf(wall[mu, kk*64:(kk+1)*64, g*512:(g+1)*512]), preferred_element_type=f32)
        if kk == 0: pre[mu, :, g*512:(g+1)*512] = r
        else: pre[mu, :, g*512:(g+1)*512] += r
    def pm_unit(u, gens):
        steps = [gi for gi in range(len(gens)) for _ in range(16 // BL)]
        n = len(steps)
        for g in range(8):
            for gi in steps[g*n//8:(g+1)*n//8]: next(gens[gi])
            pm_kh(u, g)
    def xb_prep():
        for i in range(NSEG//2):
            ab = jnp.concatenate([xB3[2*i], xB3[2*i+1]], axis=0)
            xB[8*i:8*i+8, :] = pltpu.bitcast(ab, u32)

    small = [pltpu.make_async_copy(a, b_, csem.at[i]) for i, (a, b_) in enumerate(
        ((zr_hbm, zr_ref), (F_hbm, F_ref), (skT_hbm, skT_ref), (d_hbm, d_ref), (G_hbm, G_ref), (mem_hbm, mem_ref)))]
    w_piece(0).start()
    xB_copy.start()
    for c in small: c.start()
    kf0[0:8, :] = jnp.zeros((8,128), f32); kf1[0:8, :] = jnp.zeros((8,128), f32)
    xB_copy.wait()
    for c in kvh_copies(0): c.start()
    w_piece(1).start()
    with jax.named_scope('ph1'):
        xb_prep()
        w_piece(0).wait()
        w_piece(2).start()
        repack(0)
    rng3 = (range(0,5), range(5,10), range(10,16))
    rng2 = (range(0,8), range(8,16))
    def sched(u):
        if u == 0: return None, False, []
        if u <= 21: return (u-1)//3, (u-1) % 3 == 0, rng3[(u-1) % 3]
        return 7, u == 22, rng2[u-22]
    with jax.named_scope('ph2'):
        for c in small: c.wait()
        for c in kvh_copies(0): c.wait()
        for c in kvh_copies(1): c.start()
        for u in range(24):
            j, first, cs = sched(u)
            pm_unit(u, [s2_gen(j, c) for c in cs])
            if u == 0:
                w, dd = s1_pre(0)
                for c in range(NC): s1_c(0, c, w, dd)
            else:
                if j + 1 < NT: w, dd = s1_pre(j+1)
                for c in cs:
                    if j + 1 < NT: s1_c(j+1, c, w, dd)
                    if j >= 1: s3_c(j-1, c)
            if u < 23:
                w_piece(u+1).wait()
                jn, firstn, _ = sched(u+1)
                if firstn:
                    if jn + 1 < NT:
                        for c in kvh_copies(jn+1): c.wait()
                    if jn >= 1: q_copy(jn-1).wait()
                    if jn + 2 < NT:
                        for c in kvh_copies(jn+2): c.start()
                    q_copy(jn).start()
                if u + 3 < 24: w_piece(u+3).start()
                if 1 <= u < 17 and u % 2 == 1: wo_copy((u-1)//2).start()
                if u == 18: x_piece(0, 1).start()
                repack(u+1)
        q_copy(NT-1).wait()
        for c in range(NC): s3_c(NT-1, c)
        ob_copy.start()
    for n in range(8): wo_copy(n).wait()
    x_piece(0, 1).wait()
    for p in range(1, 8): x_piece(p, 2).start()

    membuf[...] = mem_ref[...].astype(f32)
    ri = lax.broadcasted_iota(jnp.int32, (40, 40), 0)
    ci = lax.broadcasted_iota(jnp.int32, (40, 40), 1)
    mask = (ri < 8) | (ri >= ci)
    c2 = float(128 ** -0.5 * np.log2(np.e))
    wou = wo.bitcast(u32)
    def step(s, mem):
        r0 = pl.multiple_of(s * 32, 32)
        p0 = pl.multiple_of(s * 8, 8)
        xs = xb[pl.ds(r0, 32), :].astype(f32)
        h = jnp.concatenate([mem, xs[0:24]], axis=0)
        def proj(mu, g):
            cs = slice(g * 512, (g + 1) * 512)
            r = jnp.dot(h, bf(wall[mu, :, cs]), preferred_element_type=f32)
            return jnp.concatenate([r, pre[mu, pl.ds(p0, 8), cs]], axis=0)
        def scores(q, k):
            return [lax.dot_general(q[:, j*128:(j+1)*128], k[:, j*128:(j+1)*128], NT_, preferred_element_type=f32) for j in range(4)]
        def softmax(scs):
            ps = []
            for sc in scs:
                sc = jnp.where(mask, sc, -1e30)
                m = jnp.max(sc, axis=-1, keepdims=True)
                p = jnp.exp2((sc - m) * c2)
                l = jnp.sum(p, axis=-1, keepdims=True)
                r = pl.reciprocal(l, approx=True)
                r = r * (2.0 - l * r)
                ps.append(p * r)
            return ps
        def pv(ps, v, g):
            for j in range(4):
                o = jnp.dot(ps[j], v[:, j*128:(j+1)*128], preferred_element_type=f32)
                obuf[:, (g * 4 + j) * 128:(g * 4 + j + 1) * 128] = o
        def p1dots(ns):
            o1 = obuf[:, 0:3584]
            for n in ns:
                pbuf[:, n*128:(n+1)*128] = jnp.dot(o1, bf(wou[n, 0:1792, :]), preferred_element_type=f32)
        q = proj(0, 0); k = proj(1, 0); v = proj(2, 0)
        for g in range(8):
            if g + 1 < 8:
                qn = proj(0, g + 1)
                sc = scores(q, k)
                kn = proj(1, g + 1)
                ps = softmax(sc)
                vn = proj(2, g + 1)
                pv(ps, v, g)
                q, k, v = qn, kn, vn
            else:
                p1dots(range(2))
                sc = scores(q, k)
                p1dots(range(2, 5))
                ps = softmax(sc)
                pv(ps, v, g)
                p1dots(range(5, 8))
        o2 = obuf[:, 3584:4096]
        outs = [pbuf[:, n*128:(n+1)*128] + jnp.dot(o2, bf(wou[n, 1792:2048, :]), preferred_element_type=f32) for n in range(8)]
        outb = jnp.concatenate(outs, axis=1).astype(bf16)
        newmem = outb[0:8].astype(f32)
        aout[pl.ds(r0, 32), :] = outb[8:40]
        pltpu.make_async_copy(aout.at[pl.ds(r0, 32), :], out_hbm.at[pl.ds(r0, 32), pl.ds(0, D)], osem.at[1]).start()
        return newmem
    UN = 2
    def stepn(t, carry):
        @pl.when(t == (4 // UN) * 2 - 1)
        def _():
            pltpu.make_async_copy(x_hbm.at[pl.ds(256, 7*256), :], xb.at[pl.ds(256, 7*256), :], wsems.at[2]).wait()
        mem = membuf[...]
        for u in range(UN):
            mem = step(t*UN+u, mem)
        membuf[...] = mem
        return carry
    with jax.named_scope('chain'):
        lax.fori_loop(0, NSEG//UN, stepn, 0)
    ob_copy.wait()
    pltpu.make_async_copy(aout, out_hbm.at[:, pl.ds(0, D)], osem.at[1]).wait()

@jax.jit
def pallas_concat_heads__memory_aug_recurrent_mem_tr__ssm_conv_h3__prompt_kernel(A_x, A_mem0, A_Wq, A_Wk, A_Wv, A_Wo, A_seg_len, B_q, B_k, B_v, B_shift_k, B_ssm_k, B_ssm_D):
    F,G = _consts()
    any_ = pl.BlockSpec(memory_space=pl.ANY)
    vm = pl.BlockSpec(memory_space=pltpu.VMEM)
    V = pltpu.VMEM
    out = pl.pallas_call(kernel, out_shape=jax.ShapeDtypeStruct((S,2*D), bf16),
        in_specs=[any_]*16, out_specs=any_,
        scratch_shapes=[V((8,128),u32), V((8,D),bf16), V((4,D),bf16), V((D,),bf16), V((256,128),bf16), V((128,256),bf16), pltpu.SemaphoreType.DMA((6,)),
            V((S,D),bf16), V((64,8,D),bf16), V((256,D),u32), V((3,512,4096),u32),
            V((8,4096,128),bf16), V((NSTG,2048,128),u32), V((S,D),bf16), V((8,D),f32), V((40,4096),f32), V((40,1024),f32),
            V((3,512,4096),f32),
            V((2,S,128),bf16), V((2,S,128),bf16), V((2,S,128),bf16), V((2,128,S),bf16), V((S,D),bf16),
            V((NC,384,128),f32), V((NC,384,128),f32), V((NC,384,128),f32), V((NC,384,128),f32),
            V((NC,256,128),f32), V((NC,256,128),f32), V((S+8,128),f32), V((S+8,128),f32),
            pltpu.SemaphoreType.DMA((4,2)), pltpu.SemaphoreType.DMA((4,)), pltpu.SemaphoreType.DMA((NSTG,)), pltpu.SemaphoreType.DMA((2,))],
        compiler_params=pltpu.CompilerParams(vmem_limit_bytes=124*1024*1024), name="kf",
    )(jnp.asarray(np.zeros((8,128), np.uint32)), A_x.reshape(S,D), A_x.reshape(64,32,D), A_mem0.reshape(8,D), A_Wq.reshape(32768,128), A_Wk.reshape(32768,128), A_Wv.reshape(32768,128),
      A_Wo.reshape(4096,D), B_q.reshape(S,D), B_k.reshape(S,D), B_v.reshape(S,D), B_shift_k.T, B_ssm_k, B_ssm_D,
      jnp.asarray(F).astype(bf16), jnp.asarray(G).astype(bf16))
    return out.reshape(1,S,2*D)
```

```python
import jax, jax.numpy as jnp, numpy as np
from jax import lax
from jax.experimental import pallas as pl
from jax.experimental.pallas import tpu as pltpu

S=2048; D=1024; NC=16; NT=8; NSEG=64
bf16=jnp.bfloat16; f32=jnp.float32; u32=jnp.uint32

def _consts():
    k = np.arange(128)[:,None]; t = np.arange(128)[None,:]
    th = np.pi*(2*k+1)*t/256.0
    F = np.concatenate([np.cos(th), -np.sin(th)], axis=0)
    G = np.concatenate([np.cos(th).T, -np.sin(th).T], axis=1)/128.0
    if 1:
        perm = np.array([128*p + 8*g + r for g in range(16) for p in range(2) for r in range(8)])
        G = G[:, perm]
    return F.astype(np.float32), G.astype(np.float32)

def bf(x): return pltpu.bitcast(x, bf16)
NT_ = (((1,),(1,)),((),()))
NSTG = 4

def kernel(zr_hbm, x_hbm, x3_hbm, mem_hbm, wq_hbm, wk_hbm, wv_hbm, wo_hbm,
           q_hbm, k_hbm, v_hbm, skT_hbm, h_hbm, d_hbm, F_hbm, G_hbm,
           out_hbm,
           zr_ref, mem_ref, skT_ref, d_ref, F_ref, G_ref, csem, fsem,
           xb, xB3, xB, wall, wo, stg, aout, membuf, obuf, pbuf, pre,
           kb, vb, qb, hb, ob, X0, H0, X1, H1, Z0, Z1, kf0, kf1,
           sems, wsems, ssems, osem):
    def w_piece(u):
        mu, kk = u // 8, u % 8
        src = (wq_hbm, wk_hbm, wv_hbm)[mu]
        return pltpu.make_async_copy(src.at[pl.ds(kk*4096, 4096), :], stg.at[u % NSTG].bitcast(bf16), ssems.at[u % NSTG])
    def x_piece(p, sem):
        return pltpu.make_async_copy(x_hbm.at[pl.ds(p*256, 256), :], xb.at[pl.ds(p*256, 256), :], wsems.at[sem])
    def wo_copy(n):
        return pltpu.make_async_copy(wo_hbm.at[:, pl.ds(n*128,128)], wo.at[n], wsems.at[0])
    xB_copy = pltpu.make_async_copy(x3_hbm.at[:, pl.ds(24, 8), :], xB3, wsems.at[3])
    def kvh_copies(j):
        cs = pl.ds(j*128, 128); sl = j % 2
        return [pltpu.make_async_copy(k_hbm.at[:, cs], kb.at[sl], sems.at[0, sl]),
                pltpu.make_async_copy(v_hbm.at[:, cs], vb.at[sl], sems.at[1, sl]),
                pltpu.make_async_copy(h_hbm.at[cs, :], hb.at[sl], sems.at[2, sl])]
    def q_copy(j):
        return pltpu.make_async_copy(q_hbm.at[:, pl.ds(j*128, 128)], qb.at[j % 2], sems.at[3, j % 2])
    ob_copy = pltpu.make_async_copy(ob, out_hbm.at[:, pl.ds(D, D)], osem.at[0])
    sgn = jnp.where(lax.broadcasted_iota(jnp.int32,(8,128),0) % 2 == 0, 1.0, -1.0).astype(f32)

    def fence():
        pl.semaphore_signal(fsem, 1)
        pl.semaphore_wait(fsem, 1)
    def s1_pre(j):
        l0 = j*128
        w = skT_ref[:, l0:l0+128].astype(f32)
        dd = d_ref[l0:l0+128].astype(f32).reshape(1, 128)
        return [jnp.broadcast_to(w[r:r+1], (8,128)) for r in range(4)], dd
    def s1_c(j, c, w, dd):
        Xh, Hh, kf = (X0, H0, kf0) if j % 2 == 0 else (X1, H1, kf1)
        sl = j % 2
        F = F_ref[...]
        kf[8+c*128:8+(c+1)*128, :] = kb[sl, c*128:(c+1)*128, :].astype(f32)
        kvs = []
        for r in range(16):
            b = 8 + c*128 + r*8
            kvs.append(kf[b:b+8, :]*w[0] + kf[b-1:b+7, :]*w[1] + kf[b-2:b+6, :]*w[2] + kf[b-3:b+5, :]*w[3])
        kv = (jnp.concatenate(kvs, axis=0) * vb[sl, c*128:(c+1)*128, :].astype(f32)).astype(bf16)
        xh = jnp.dot(F, kv, preferred_element_type=f32)
        hh = lax.dot_general(F, hb[sl, :, c*128:(c+1)*128], NT_, preferred_element_type=f32)
        e = hh[0:128]; f = hh[128:256]
        if c == 0: e = e + dd
        Xh[c, 0:256, :] = xh
        Hh[c, 0:128, :] = e
        if 0:
            Xh[c, 256:384, :] = xh[0:128] + xh[128:256]
            Hh[c, 128:256, :] = f - e
            Hh[c, 256:384, :] = e + f
        else:
            Hh[c, 128:256, :] = f
    BL = 4
    HK = []
    def s2_gen(j, g):
        Xh, Hh, Zb = (X0, H0, Z0) if j % 2 == 0 else (X1, H1, Z1)
        r0 = g*8; r1 = g*8+128; r2 = g*8+256
        M3 = 0
        def X(c): return (Xh[c, r0:r0+8, :], Xh[c, r1:r1+8, :], Xh[c, r2:r2+8, :]) if M3 else (Xh[c, r0:r0+8, :], Xh[c, r1:r1+8, :], None)
        def H(m): return (Hh[m, r0:r0+8, :], Hh[m, r1:r1+8, :], Hh[m, r2:r2+8, :]) if M3 else (Hh[m, r0:r0+8, :], Hh[m, r1:r1+8, :], None)
        prev = None
        for b in range(16//BL):
            acc = [None]*BL
            for m in range(BL*b+BL):
                he, hfe, hef = H(m)
                for i in range(BL):
                    c = BL*b+i
                    if m > c: continue
                    xa, xb_, xs_ = X(c-m)
                    p = (he*xs_, xa*hfe, xb_*hef) if M3 else (xa*he - xb_*hfe, xa*hfe + xb_*he)
                    acc[i] = p if acc[i] is None else tuple(a_+p_ for a_, p_ in zip(acc[i], p))
            for i in range(BL):
                c = BL*b+i
                yr, yi = (acc[i][0] - acc[i][2], acc[i][0] + acc[i][1]) if M3 else acc[i]
                if prev is None: zr, zi = yr, yi
                else: zr, zi = yr - sgn*prev[1], yi + sgn*prev[0]
                prev = (yr, yi)
                if 1:
                    zp = pltpu.bitcast(jnp.concatenate([zr, zi], axis=0).astype(bf16), u32)
                    Zb[c, r0:r0+8, :] = zp
                    HK.append(zp)
                else:
                    Zb[c, r0:r0+8, :] = zr; Zb[c, r1:r1+8, :] = zi
                    HK.append(pltpu.bitcast(zr, u32) | pltpu.bitcast(zi, u32))
            yield None
    def s3_c(j, c):
        Zb = Z0 if j % 2 == 0 else Z1
        G = G_ref[...]
        y = jnp.dot(G, bf(Zb[c]) if 1 else Zb[c].astype(bf16), preferred_element_type=f32)
        rs = slice(c*128,(c+1)*128)
        ob[rs, j*128:(j+1)*128] = (qb[j % 2, rs, :].astype(f32) * y).astype(bf16)

    def repack(u):
        mu, kk = u // 8, u % 8
        sl = u % NSTG
        for i in range(8):
            for j in range(16):
                Ev = stg[sl, pl.ds(256*i + j, 8, stride=32), :]
                Ov = stg[sl, pl.ds(256*i + 16 + j, 8, stride=32), :]
                r0 = kk*64 + 8*i
                wall[mu, r0:r0+8, 256*j:256*j+128] = (Ev & 0xffff) | (Ov << 16)
                wall[mu, r0:r0+8, 256*j+128:256*j+256] = (Ev >> 16) | (Ov & jnp.uint32(0xffff0000))
    def pm_kh(u, g):
        mu, kk = u // 8, u % 8
        pieces = [xB[8*r:8*r+8, 128*kk:128*kk+128] for r in range(32)]
        n = len(HK)
        if n:
            z = zr_ref[...]
            for i, hk in enumerate(HK):
                rg = (i * 32) // n
                pieces[rg] = pieces[rg] | (hk & z)
            HK.clear()
        lhs = jnp.concatenate(pieces, axis=0)
        r = jnp.dot(bf(lhs), bf(wall[mu, kk*64:(kk+1)*64, g*512:(g+1)*512]), preferred_element_type=f32)
        if kk == 0: pre[mu, :, g*512:(g+1)*512] = r
        else: pre[mu, :, g*512:(g+1)*512] += r
    def pm_unit(u, gens):
        steps = [gi for gi in range(len(gens)) for _ in range(16 // BL)]
        n = len(steps)
        for g in range(8):
            for gi in steps[g*n//8:(g+1)*n//8]: next(gens[gi])
            pm_kh(u, g)
    def xb_prep():
        for i in range(NSEG//2):
            ab = jnp.concatenate([xB3[2*i], xB3[2*i+1]], axis=0)
            xB[8*i:8*i+8, :] = pltpu.bitcast(ab, u32)

    small = [pltpu.make_async_copy(a, b_, csem.at[i]) for i, (a, b_) in enumerate(
        ((zr_hbm, zr_ref), (F_hbm, F_ref), (skT_hbm, skT_ref), (d_hbm, d_ref), (G_hbm, G_ref), (mem_hbm, mem_ref)))]
    w_piece(0).start()
    xB_copy.start()
    for c in small: c.start()
    kf0[0:8, :] = jnp.zeros((8,128), f32); kf1[0:8, :] = jnp.zeros((8,128), f32)
    w_piece(0).wait()
    for c in kvh_copies(0): c.start()
    w_piece(1).start()
    for c in kvh_copies(1): c.start()
    w_piece(2).start()
    if 1 & 1: fence()
    with jax.named_scope('ph1'):
        repack(0)
        xB_copy.wait()
        xb_prep()
    rng3 = (range(0,5), range(5,10), range(10,16))
    rng2 = (range(0,8), range(8,16))
    def sched(u):
        if u == 0: return None, False, []
        if u <= 21: return (u-1)//3, (u-1) % 3 == 0, rng3[(u-1) % 3]
        return 7, u == 22, rng2[u-22]
    with jax.named_scope('ph2'):
        for u in range(24):
            j, first, cs = sched(u)
            pm_unit(u, [s2_gen(j, c) for c in cs])
            if u == 0:
                for c in small: c.wait()
                for c in kvh_copies(0): c.wait()
                w, dd = s1_pre(0)
                for c in range(NC): s1_c(0, c, w, dd)
            else:
                if u == 1:
                    for c in kvh_copies(1): c.wait()
                if j + 1 < NT: w, dd = s1_pre(j+1)
                if 0 == 0:
                    for c in cs:
                        if j + 1 < NT: s1_c(j+1, c, w, dd)
                        if j >= 1: s3_c(j-1, c)
                elif 0 == 1:
                    for c in cs:
                        if j + 1 < NT: s1_c(j+1, c, w, dd)
                    for c in cs:
                        if j >= 1: s3_c(j-1, c)
                else:
                    for c in cs:
                        if j >= 1: s3_c(j-1, c)
                    for c in cs:
                        if j + 1 < NT: s1_c(j+1, c, w, dd)
            if u < 23:
                w_piece(u+1).wait()
                jn, firstn, _ = sched(u+1)
                if firstn:
                    if jn + 1 < NT and jn > 0:
                        for c in kvh_copies(jn+1): c.wait()
                    if jn >= 1: q_copy(jn-1).wait()
                    if jn + 2 < NT:
                        for c in kvh_copies(jn+2): c.start()
                    q_copy(jn).start()
                if u + 3 < 24: w_piece(u+3).start()
                if 1 <= u < 17 and u % 2 == 1: wo_copy((u-1)//2).start()
                if u == 18: x_piece(0, 1).start()
                if 1 & 2: fence()
                repack(u+1)
        q_copy(NT-1).wait()
        for c in range(NC): s3_c(NT-1, c)
        ob_copy.start()
    for n in range(8): wo_copy(n).wait()
    x_piece(0, 1).wait()
    for p in range(1, 8): x_piece(p, 2).start()

    membuf[...] = mem_ref[...].astype(f32)
    ri = lax.broadcasted_iota(jnp.int32, (40, 40), 0)
    ci = lax.broadcasted_iota(jnp.int32, (40, 40), 1)
    mask = (ri < 8) | (ri >= ci)
    c2 = float(128 ** -0.5 * np.log2(np.e))
    wou = wo.bitcast(u32)
    def step(s, mem):
        r0 = pl.multiple_of(s * 32, 32)
        p0 = pl.multiple_of(s * 8, 8)
        xs = xb[pl.ds(r0, 32), :].astype(f32)
        h = jnp.concatenate([mem, xs[0:24]], axis=0)
        def proj(mu, g):
            cs = slice(g * 512, (g + 1) * 512)
            r = jnp.dot(h, bf(wall[mu, :, cs]), preferred_element_type=f32)
            return jnp.concatenate([r, pre[mu, pl.ds(p0, 8), cs]], axis=0)
        def scores(q, k):
            return [lax.dot_general(q[:, j*128:(j+1)*128], k[:, j*128:(j+1)*128], NT_, preferred_element_type=f32) for j in range(4)]
        def softmax(scs):
            ps = []
            for sc in scs:
                sc = jnp.where(mask, sc, -1e30)
                m = jnp.max(sc, axis=-1, keepdims=True)
                p = jnp.exp2((sc - m) * c2)
                l = jnp.sum(p, axis=-1, keepdims=True)
                r = pl.reciprocal(l, approx=True)
                r = r * (2.0 - l * r)
                ps.append(p * r)
            return ps
        def pv(ps, v, g):
            for j in range(4):
                o = jnp.dot(ps[j], v[:, j*128:(j+1)*128], preferred_element_type=f32)
                obuf[:, (g * 4 + j) * 128:(g * 4 + j + 1) * 128] = o
        def p1dots(ns):
            o1 = obuf[:, 0:3584]
            for n in ns:
                pbuf[:, n*128:(n+1)*128] = jnp.dot(o1, bf(wou[n, 0:1792, :]), preferred_element_type=f32)
        q = proj(0, 0); k = proj(1, 0); v = proj(2, 0)
        for g in range(8):
            if g + 1 < 8:
                qn = proj(0, g + 1)
                sc = scores(q, k)
                kn = proj(1, g + 1)
                ps = softmax(sc)
                vn = proj(2, g + 1)
                pv(ps, v, g)
                q, k, v = qn, kn, vn
            else:
                p1dots(range(2))
                sc = scores(q, k)
                p1dots(range(2, 5))
                ps = softmax(sc)
                pv(ps, v, g)
                p1dots(range(5, 8))
        o2 = obuf[:, 3584:4096]
        outs = [pbuf[:, n*128:(n+1)*128] + jnp.dot(o2, bf(wou[n, 1792:2048, :]), preferred_element_type=f32) for n in range(8)]
        outb = jnp.concatenate(outs, axis=1).astype(bf16)
        newmem = outb[0:8].astype(f32)
        aout[pl.ds(r0, 32), :] = outb[8:40]
        pltpu.make_async_copy(aout.at[pl.ds(r0, 32), :], out_hbm.at[pl.ds(r0, 32), pl.ds(0, D)], osem.at[1]).start()
        return newmem
    UN = 2
    def stepn(t, carry):
        @pl.when(t == (4 // UN) * 2 - 1)
        def _():
            pltpu.make_async_copy(x_hbm.at[pl.ds(256, 7*256), :], xb.at[pl.ds(256, 7*256), :], wsems.at[2]).wait()
        mem = membuf[...]
        for u in range(UN):
            mem = step(t*UN+u, mem)
        membuf[...] = mem
        return carry
    with jax.named_scope('chain'):
        lax.fori_loop(0, NSEG//UN, stepn, 0)
    ob_copy.wait()
    pltpu.make_async_copy(aout, out_hbm.at[:, pl.ds(0, D)], osem.at[1]).wait()

@jax.jit
def pallas_concat_heads__memory_aug_recurrent_mem_tr__ssm_conv_h3__prompt_kernel(A_x, A_mem0, A_Wq, A_Wk, A_Wv, A_Wo, A_seg_len, B_q, B_k, B_v, B_shift_k, B_ssm_k, B_ssm_D):
    F,G = _consts()
    any_ = pl.BlockSpec(memory_space=pl.ANY)
    vm = pl.BlockSpec(memory_space=pltpu.VMEM)
    V = pltpu.VMEM
    out = pl.pallas_call(kernel, out_shape=jax.ShapeDtypeStruct((S,2*D), bf16),
        in_specs=[any_]*16, out_specs=any_,
        scratch_shapes=[V((8,128),u32), V((8,D),bf16), V((4,D),bf16), V((D,),bf16), V((256,128),bf16), V((128,256),bf16), pltpu.SemaphoreType.DMA((6,)), pltpu.SemaphoreType.REGULAR,
            V((S,D),bf16), V((64,8,D),bf16), V((256,D),u32), V((3,512,4096),u32),
            V((8,4096,128),bf16), V((NSTG,2048,128),u32), V((S,D),bf16), V((8,D),f32), V((40,4096),f32), V((40,1024),f32),
            V((3,512,4096),f32),
            V((2,S,128),bf16), V((2,S,128),bf16), V((2,S,128),bf16), V((2,128,S),bf16), V((S,D),bf16),
            V((NC,384,128),f32), V((NC,384,128),f32), V((NC,384,128),f32), V((NC,384,128),f32),
            *([V((NC,128,128),u32) if 1 else V((NC,256,128),f32)]*2), V((S+8,128),f32), V((S+8,128),f32),
            pltpu.SemaphoreType.DMA((4,2)), pltpu.SemaphoreType.DMA((4,)), pltpu.SemaphoreType.DMA((NSTG,)), pltpu.SemaphoreType.DMA((2,))],
        compiler_params=pltpu.CompilerParams(vmem_limit_bytes=124*1024*1024), name="kf",
    )(jnp.asarray(np.zeros((8,128), np.uint32)), A_x.reshape(S,D), A_x.reshape(64,32,D), A_mem0.reshape(8,D), A_Wq.reshape(32768,128), A_Wk.reshape(32768,128), A_Wv.reshape(32768,128),
      A_Wo.reshape(4096,D), B_q.reshape(S,D), B_k.reshape(S,D), B_v.reshape(S,D), B_shift_k.T, B_ssm_k, B_ssm_D,
      jnp.asarray(F).astype(bf16), jnp.asarray(G).astype(bf16))
    return out.reshape(1,S,2*D)
```

```python
import jax, jax.numpy as jnp, numpy as np
from jax import lax
from jax.experimental import pallas as pl
from jax.experimental.pallas import tpu as pltpu

S=2048; D=1024; NC=16; NT=8; NSEG=64
bf16=jnp.bfloat16; f32=jnp.float32; u32=jnp.uint32

def _consts():
    k = np.arange(128)[:,None]; t = np.arange(128)[None,:]
    th = np.pi*(2*k+1)*t/256.0
    F = np.concatenate([np.cos(th), -np.sin(th)], axis=0)
    G = np.concatenate([np.cos(th).T, -np.sin(th).T], axis=1)/128.0
    if 1:
        perm = np.array([128*p + 8*g + r for g in range(16) for p in range(2) for r in range(8)])
        G = G[:, perm]
    return F.astype(np.float32), G.astype(np.float32)

def bf(x): return pltpu.bitcast(x, bf16)
NT_ = (((1,),(1,)),((),()))
NSTG = 4

def kernel(zr_hbm, x_hbm, x3_hbm, mem_hbm, wq_hbm, wk_hbm, wv_hbm, wo_hbm,
           q_hbm, k_hbm, v_hbm, skT_hbm, h_hbm, d_hbm, F_hbm, G_hbm,
           out_hbm,
           zr_ref, mem_ref, skT_ref, d_ref, F_ref, G_ref, csem, fsem,
           xb, xB3, xB, wall, wo, stg, aout, membuf, obuf, pbuf, pre,
           kb, vb, qb, hb, ob, X0, H0, X1, H1, Z0, Z1, kf0, kf1,
           sems, wsems, ssems, osem):
    def w_piece(u):
        mu, kk = u // 8, u % 8
        src = (wq_hbm, wk_hbm, wv_hbm)[mu]
        return pltpu.make_async_copy(src.at[pl.ds(kk*4096, 4096), :], stg.at[u % NSTG].bitcast(bf16), ssems.at[u % NSTG])
    def x_piece(p, sem):
        return pltpu.make_async_copy(x_hbm.at[pl.ds(p*256, 256), :], xb.at[pl.ds(p*256, 256), :], wsems.at[sem])
    def wo_copy(n):
        return pltpu.make_async_copy(wo_hbm.at[:, pl.ds(n*128,128)], wo.at[n], wsems.at[0])
    xB_copy = pltpu.make_async_copy(x3_hbm.at[:, pl.ds(24, 8), :], xB3, wsems.at[3])
    def kvh_copies(j):
        cs = pl.ds(j*128, 128); sl = j % 2
        return [pltpu.make_async_copy(k_hbm.at[:, cs], kb.at[sl], sems.at[0, sl]),
                pltpu.make_async_copy(v_hbm.at[:, cs], vb.at[sl], sems.at[1, sl]),
                pltpu.make_async_copy(h_hbm.at[cs, :], hb.at[sl], sems.at[2, sl])]
    def q_copy(j):
        return pltpu.make_async_copy(q_hbm.at[:, pl.ds(j*128, 128)], qb.at[j % 2], sems.at[3, j % 2])
    ob_copy = pltpu.make_async_copy(ob, out_hbm.at[:, pl.ds(D, D)], osem.at[0])
    sgn = jnp.where(lax.broadcasted_iota(jnp.int32,(8,128),0) % 2 == 0, 1.0, -1.0).astype(f32)

    def fence():
        pl.semaphore_signal(fsem, 1)
        pl.semaphore_wait(fsem, 1)
    def s1_pre(j):
        l0 = j*128
        w = skT_ref[:, l0:l0+128].astype(f32)
        dd = d_ref[l0:l0+128].astype(f32).reshape(1, 128)
        return [jnp.broadcast_to(w[r:r+1], (8,128)) for r in range(4)], dd
    def s1_c(j, c, w, dd):
        Xh, Hh, kf = (X0, H0, kf0) if j % 2 == 0 else (X1, H1, kf1)
        sl = j % 2
        F = F_ref[...]
        kf[8+c*128:8+(c+1)*128, :] = kb[sl, c*128:(c+1)*128, :].astype(f32)
        kvs = []
        for r in range(16):
            b = 8 + c*128 + r*8
            kvs.append(kf[b:b+8, :]*w[0] + kf[b-1:b+7, :]*w[1] + kf[b-2:b+6, :]*w[2] + kf[b-3:b+5, :]*w[3])
        kv = (jnp.concatenate(kvs, axis=0) * vb[sl, c*128:(c+1)*128, :].astype(f32)).astype(bf16)
        xh = jnp.dot(F, kv, preferred_element_type=f32)
        hh = lax.dot_general(F, hb[sl, :, c*128:(c+1)*128], NT_, preferred_element_type=f32)
        e = hh[0:128]; f = hh[128:256]
        if c == 0: e = e + dd
        Xh[c, 0:256, :] = xh
        Hh[c, 0:128, :] = e
        if 0:
            Xh[c, 256:384, :] = xh[0:128] + xh[128:256]
            Hh[c, 128:256, :] = f - e
            Hh[c, 256:384, :] = e + f
        else:
            Hh[c, 128:256, :] = f
    BL = 4
    HK = []
    def s2_gen(j, g):
        Xh, Hh, Zb = (X0, H0, Z0) if j % 2 == 0 else (X1, H1, Z1)
        r0 = g*8; r1 = g*8+128; r2 = g*8+256
        M3 = 0
        def X(c): return (Xh[c, r0:r0+8, :], Xh[c, r1:r1+8, :], Xh[c, r2:r2+8, :]) if M3 else (Xh[c, r0:r0+8, :], Xh[c, r1:r1+8, :], None)
        def H(m): return (Hh[m, r0:r0+8, :], Hh[m, r1:r1+8, :], Hh[m, r2:r2+8, :]) if M3 else (Hh[m, r0:r0+8, :], Hh[m, r1:r1+8, :], None)
        prev = None
        for b in range(16//BL):
            acc = [None]*BL
            for m in range(BL*b+BL):
                he, hfe, hef = H(m)
                for i in range(BL):
                    c = BL*b+i
                    if m > c: continue
                    xa, xb_, xs_ = X(c-m)
                    p = (he*xs_, xa*hfe, xb_*hef) if M3 else (xa*he - xb_*hfe, xa*hfe + xb_*he)
                    acc[i] = p if acc[i] is None else tuple(a_+p_ for a_, p_ in zip(acc[i], p))
            for i in range(BL):
                c = BL*b+i
                yr, yi = (acc[i][0] - acc[i][2], acc[i][0] + acc[i][1]) if M3 else acc[i]
                if prev is None: zr, zi = yr, yi
                else: zr, zi = yr - sgn*prev[1], yi + sgn*prev[0]
                prev = (yr, yi)
                if 1:
                    zp = pltpu.bitcast(jnp.concatenate([zr, zi], axis=0).astype(bf16), u32)
                    Zb[c, r0:r0+8, :] = zp
                    HK.append(zp)
                else:
                    Zb[c, r0:r0+8, :] = zr; Zb[c, r1:r1+8, :] = zi
                    HK.append(pltpu.bitcast(zr, u32) | pltpu.bitcast(zi, u32))
            yield None
    def s3_c(j, c):
        Zb = Z0 if j % 2 == 0 else Z1
        G = G_ref[...]
        y = jnp.dot(G, bf(Zb[c]) if 1 else Zb[c].astype(bf16), preferred_element_type=f32)
        rs = slice(c*128,(c+1)*128)
        ob[rs, j*128:(j+1)*128] = (qb[j % 2, rs, :].astype(f32) * y).astype(bf16)

    def s1_q(j, cq, w, dd):
        Xh, Hh, kf = (X0, H0, kf0) if j % 2 == 0 else (X1, H1, kf1)
        sl = j % 2
        F = F_ref[...]
        kvl = []
        for c in range(4*cq, 4*cq+4):
            kf[8+c*128:8+(c+1)*128, :] = kb[sl, c*128:(c+1)*128, :].astype(f32)
            kvs = []
            for r in range(16):
                b = 8 + c*128 + r*8
                kvs.append(kf[b:b+8, :]*w[0] + kf[b-1:b+7, :]*w[1] + kf[b-2:b+6, :]*w[2] + kf[b-3:b+5, :]*w[3])
            kvl.append((jnp.concatenate(kvs, axis=0) * vb[sl, c*128:(c+1)*128, :].astype(f32)).astype(bf16))
        xh4 = jnp.dot(F, jnp.concatenate(kvl, axis=1), preferred_element_type=f32)
        hcat = jnp.concatenate([hb[sl, :, c*128:(c+1)*128] for c in range(4*cq, 4*cq+4)], axis=0)
        hh4 = lax.dot_general(F, hcat, NT_, preferred_element_type=f32)
        for i, c in enumerate(range(4*cq, 4*cq+4)):
            xh = xh4[:, i*128:(i+1)*128]; hh = hh4[:, i*128:(i+1)*128]
            e = hh[0:128]; f = hh[128:256]
            if c == 0: e = e + dd
            Xh[c, 0:256, :] = xh
            Hh[c, 0:128, :] = e
            if 0:
                Xh[c, 256:384, :] = xh[0:128] + xh[128:256]
                Hh[c, 128:256, :] = f - e
                Hh[c, 256:384, :] = e + f
            else:
                Hh[c, 128:256, :] = f
    def s3_q(j, cq):
        Zb = Z0 if j % 2 == 0 else Z1
        G = G_ref[...]
        z4 = jnp.concatenate([Zb[c] for c in range(4*cq, 4*cq+4)], axis=1)
        y4 = jnp.dot(G, bf(z4), preferred_element_type=f32)
        for i, c in enumerate(range(4*cq, 4*cq+4)):
            rs = slice(c*128,(c+1)*128)
            ob[rs, j*128:(j+1)*128] = (qb[j % 2, rs, :].astype(f32) * y4[:, i*128:(i+1)*128]).astype(bf16)
    def repack(u):
        mu, kk = u // 8, u % 8
        sl = u % NSTG
        for i in range(8):
            for j in range(16):
                Ev = stg[sl, pl.ds(256*i + j, 8, stride=32), :]
                Ov = stg[sl, pl.ds(256*i + 16 + j, 8, stride=32), :]
                r0 = kk*64 + 8*i
                wall[mu, r0:r0+8, 256*j:256*j+128] = (Ev & 0xffff) | (Ov << 16)
                wall[mu, r0:r0+8, 256*j+128:256*j+256] = (Ev >> 16) | (Ov & jnp.uint32(0xffff0000))
    def pm_kh(u, g):
        mu, kk = u // 8, u % 8
        pieces = [xB[8*r:8*r+8, 128*kk:128*kk+128] for r in range(32)]
        n = len(HK)
        if n:
            z = zr_ref[...]
            for i, hk in enumerate(HK):
                rg = 0 + (i * (32-0)) // n
                pieces[rg] = pieces[rg] | (hk & z)
            HK.clear()
        lhs = jnp.concatenate(pieces, axis=0)
        r = jnp.dot(bf(lhs), bf(wall[mu, kk*64:(kk+1)*64, g*512:(g+1)*512]), preferred_element_type=f32)
        if kk == 0: pre[mu, :, g*512:(g+1)*512] = r
        else: pre[mu, :, g*512:(g+1)*512] += r
    def pm_unit(u, gens):
        steps = [gi for gi in range(len(gens)) for _ in range(16 // BL)]
        n = len(steps)
        for g in range(8):
            for gi in steps[g*n//8:(g+1)*n//8]: next(gens[gi])
            pm_kh(u, g)
    def xb_prep():
        for i in range(NSEG//2):
            ab = jnp.concatenate([xB3[2*i], xB3[2*i+1]], axis=0)
            xB[8*i:8*i+8, :] = pltpu.bitcast(ab, u32)

    small = [pltpu.make_async_copy(a, b_, csem.at[i]) for i, (a, b_) in enumerate(
        ((zr_hbm, zr_ref), (F_hbm, F_ref), (skT_hbm, skT_ref), (d_hbm, d_ref), (G_hbm, G_ref), (mem_hbm, mem_ref)))]
    w_piece(0).start()
    xB_copy.start()
    for c in small: c.start()
    kf0[0:8, :] = jnp.zeros((8,128), f32); kf1[0:8, :] = jnp.zeros((8,128), f32)
    w_piece(0).wait()
    for c in kvh_copies(0): c.start()
    w_piece(1).start()
    for c in kvh_copies(1): c.start()
    w_piece(2).start()
    if 1 & 1: fence()
    with jax.named_scope('ph1'):
        repack(0)
        xB_copy.wait()
        xb_prep()
    QD = 0
    rng3 = (range(0,4), range(4,8), range(8,16)) if QD else (range(0,5), range(5,10), range(10,16))
    rng2 = (range(0,8), range(8,16))
    def sched(u):
        if u == 0: return None, False, []
        if u <= 21: return (u-1)//3, (u-1) % 3 == 0, rng3[(u-1) % 3]
        return 7, u == 22, rng2[u-22]
    with jax.named_scope('ph2'):
        for u in range(24):
            j, first, cs = sched(u)
            pm_unit(u, [s2_gen(j, c) for c in cs])
            if 0: fence()
            if u == 0:
                for c in small: c.wait()
                for c in kvh_copies(0): c.wait()
                w, dd = s1_pre(0)
                if QD:
                    for cq in range(4): s1_q(0, cq, w, dd)
                else:
                    for c in range(NC): s1_c(0, c, w, dd)
            else:
                if u == 1:
                    for c in kvh_copies(1): c.wait()
                if j + 1 < NT: w, dd = s1_pre(j+1)
                if QD:
                    for cq in range(cs[0]//4, (cs[-1]+1)//4):
                        if j + 1 < NT: s1_q(j+1, cq, w, dd)
                        if j >= 1: s3_q(j-1, cq)
                elif 0 == 0:
                    for c in cs:
                        if j + 1 < NT: s1_c(j+1, c, w, dd)
                        if j >= 1: s3_c(j-1, c)
                elif 0 == 1:
                    for c in cs:
                        if j + 1 < NT: s1_c(j+1, c, w, dd)
                    for c in cs:
                        if j >= 1: s3_c(j-1, c)
                else:
                    for c in cs:
                        if j >= 1: s3_c(j-1, c)
                    for c in cs:
                        if j + 1 < NT: s1_c(j+1, c, w, dd)
            if u < 23:
                w_piece(u+1).wait()
                jn, firstn, _ = sched(u+1)
                if firstn:
                    if jn + 1 < NT and jn > 0:
                        for c in kvh_copies(jn+1): c.wait()
                    if jn >= 1: q_copy(jn-1).wait()
                    if jn + 2 < NT:
                        for c in kvh_copies(jn+2): c.start()
                    q_copy(jn).start()
                if u + 3 < 24: w_piece(u+3).start()
                if 1 <= u < 17 and u % 2 == 1: wo_copy((u-1)//2).start()
                if u == 18: x_piece(0, 1).start()
                if 1 & 2: fence()
                repack(u+1)
        q_copy(NT-1).wait()
        if QD:
            for cq in range(4): s3_q(NT-1, cq)
        else:
            for c in range(NC): s3_c(NT-1, c)
        ob_copy.start()
    for n in range(8): wo_copy(n).wait()
    x_piece(0, 1).wait()
    for p in range(1, 8): x_piece(p, 2).start()

    membuf[...] = mem_ref[...].astype(f32)
    ri = lax.broadcasted_iota(jnp.int32, (40, 40), 0)
    ci = lax.broadcasted_iota(jnp.int32, (40, 40), 1)
    mask = (ri < 8) | (ri >= ci)
    c2 = float(128 ** -0.5 * np.log2(np.e))
    wou = wo.bitcast(u32)
    def step(s, mem):
        r0 = pl.multiple_of(s * 32, 32)
        p0 = pl.multiple_of(s * 8, 8)
        if 2 == 1:
            h = jnp.concatenate([mem.astype(bf16), xb[pl.ds(r0, 24), :]], axis=0)
        else:
            xs = xb[pl.ds(r0, 32), :].astype(f32)
            h = jnp.concatenate([mem, xs[0:24]], axis=0).astype(bf16)
        def proj(mu, g):
            cs = slice(g * 512, (g + 1) * 512)
            r = jnp.dot(h, bf(wall[mu, :, cs]), preferred_element_type=f32)
            return jnp.concatenate([r, pre[mu, pl.ds(p0, 8), cs]], axis=0)
        def scores(q, k):
            return [lax.dot_general(q[:, j*128:(j+1)*128], k[:, j*128:(j+1)*128], NT_, preferred_element_type=f32) for j in range(4)]
        def softmax(scs):
            ps = []
            for sc in scs:
                sc = jnp.where(mask, sc, -1e30)
                m = jnp.max(sc, axis=-1, keepdims=True)
                p = jnp.exp2((sc - m) * c2)
                l = jnp.sum(p, axis=-1, keepdims=True)
                r = pl.reciprocal(l, approx=True)
                r = r * (2.0 - l * r)
                ps.append(p * r)
            return ps
        def pv(ps, v, g):
            for j in range(4):
                o = jnp.dot(ps[j], v[:, j*128:(j+1)*128], preferred_element_type=f32)
                obuf[:, (g * 4 + j) * 128:(g * 4 + j + 1) * 128] = o
        def p1dots(ns):
            o1 = obuf[:, 0:3584]
            for n in ns:
                pbuf[:, n*128:(n+1)*128] = jnp.dot(o1, bf(wou[n, 0:1792, :]), preferred_element_type=f32)
        q = proj(0, 0); k = proj(1, 0); v = proj(2, 0)
        for g in range(8):
            if g + 1 < 8:
                qn = proj(0, g + 1)
                sc = scores(q, k)
                kn = proj(1, g + 1)
                ps = softmax(sc)
                vn = proj(2, g + 1)
                pv(ps, v, g)
                q, k, v = qn, kn, vn
            else:
                p1dots(range(2))
                sc = scores(q, k)
                p1dots(range(2, 5))
                ps = softmax(sc)
                pv(ps, v, g)
                p1dots(range(5, 8))
        o2 = obuf[:, 3584:4096]
        outs = [pbuf[:, n*128:(n+1)*128] + jnp.dot(o2, bf(wou[n, 1792:2048, :]), preferred_element_type=f32) for n in range(8)]
        outb = jnp.concatenate(outs, axis=1).astype(bf16)
        newmem = outb[0:8].astype(f32)
        aout[pl.ds(r0, 32), :] = outb[8:40]
        pltpu.make_async_copy(aout.at[pl.ds(r0, 32), :], out_hbm.at[pl.ds(r0, 32), pl.ds(0, D)], osem.at[1]).start()
        return newmem
    UN = 2
    def stepn(t, carry):
        @pl.when(t == (4 // UN) * 2 - 1)
        def _():
            pltpu.make_async_copy(x_hbm.at[pl.ds(256, 7*256), :], xb.at[pl.ds(256, 7*256), :], wsems.at[2]).wait()
        mem = membuf[...]
        for u in range(UN):
            mem = step(t*UN+u, mem)
        membuf[...] = mem
        return carry
    with jax.named_scope('chain'):
        lax.fori_loop(0, NSEG//UN, stepn, 0)
    ob_copy.wait()
    pltpu.make_async_copy(aout, out_hbm.at[:, pl.ds(0, D)], osem.at[1]).wait()

@jax.jit
def pallas_concat_heads__memory_aug_recurrent_mem_tr__ssm_conv_h3__prompt_kernel(A_x, A_mem0, A_Wq, A_Wk, A_Wv, A_Wo, A_seg_len, B_q, B_k, B_v, B_shift_k, B_ssm_k, B_ssm_D):
    F,G = _consts()
    any_ = pl.BlockSpec(memory_space=pl.ANY)
    vm = pl.BlockSpec(memory_space=pltpu.VMEM)
    V = pltpu.VMEM
    out = pl.pallas_call(kernel, out_shape=jax.ShapeDtypeStruct((S,2*D), bf16),
        in_specs=[any_]*16, out_specs=any_,
        scratch_shapes=[V((8,128),u32), V((8,D),bf16), V((4,D),bf16), V((D,),bf16), V((256,128),bf16), V((128,256),bf16), pltpu.SemaphoreType.DMA((6,)), pltpu.SemaphoreType.REGULAR,
            V((S,D),bf16), V((64,8,D),bf16), V((256,D),u32), V((3,512,4096),u32),
            V((8,4096,128),bf16), V((NSTG,2048,128),u32), V((S,D),bf16), V((8,D),f32), V((40,4096),f32), V((40,1024),f32),
            V((3,512,4096),f32),
            V((2,S,128),bf16), V((2,S,128),bf16), V((2,S,128),bf16), V((2,128,S),bf16), V((S,D),bf16),
            V((NC,384,128),f32), V((NC,384,128),f32), V((NC,384,128),f32), V((NC,384,128),f32),
            *([V((NC,128,128),u32) if 1 else V((NC,256,128),f32)]*2), V((S+8,128),f32), V((S+8,128),f32),
            pltpu.SemaphoreType.DMA((4,2)), pltpu.SemaphoreType.DMA((4,)), pltpu.SemaphoreType.DMA((NSTG,)), pltpu.SemaphoreType.DMA((2,))],
        compiler_params=pltpu.CompilerParams(vmem_limit_bytes=124*1024*1024), name="kf",
    )(jnp.asarray(np.zeros((8,128), np.uint32)), A_x.reshape(S,D), A_x.reshape(64,32,D), A_mem0.reshape(8,D), A_Wq.reshape(32768,128), A_Wk.reshape(32768,128), A_Wv.reshape(32768,128),
      A_Wo.reshape(4096,D), B_q.reshape(S,D), B_k.reshape(S,D), B_v.reshape(S,D), B_shift_k.T, B_ssm_k, B_ssm_D,
      jnp.asarray(F).astype(bf16), jnp.asarray(G).astype(bf16))
    return out.reshape(1,S,2*D)
```

```python
import jax, jax.numpy as jnp, numpy as np
from jax import lax
from jax.experimental import pallas as pl
from jax.experimental.pallas import tpu as pltpu

S=2048; D=1024; NC=16; NT=8; NSEG=64
bf16=jnp.bfloat16; f32=jnp.float32; u32=jnp.uint32

def _consts():
    k = np.arange(128)[:,None]; t = np.arange(128)[None,:]
    th = np.pi*(2*k+1)*t/256.0
    F = np.concatenate([np.cos(th), -np.sin(th)], axis=0)
    G = np.concatenate([np.cos(th).T, -np.sin(th).T], axis=1)/128.0
    if 1:
        perm = np.array([128*p + 8*g + r for g in range(16) for p in range(2) for r in range(8)])
        G = G[:, perm]
    return F.astype(np.float32), G.astype(np.float32)

def bf(x): return pltpu.bitcast(x, bf16)
NT_ = (((1,),(1,)),((),()))
NSTG = 4

def kernel(zr_hbm, x_hbm, x3_hbm, mem_hbm, wq_hbm, wk_hbm, wv_hbm, wo_hbm,
           q_hbm, k_hbm, v_hbm, skT_hbm, h_hbm, d_hbm, F_hbm, G_hbm,
           out_hbm,
           zr_ref, mem_ref, skT_ref, d_ref, F_ref, G_ref, csem, fsem,
           xb, xB3, xB, wall, wo, stg, aout, membuf, obuf, pbuf, pre,
           kb, vb, qb, hb, ob, X0, H0, X1, H1, Z0, Z1, kf0, kf1,
           sems, wsems, ssems, osem):
    def w_piece(u):
        mu, kk = u // 8, u % 8
        src = (wq_hbm, wk_hbm, wv_hbm)[mu]
        return pltpu.make_async_copy(src.at[pl.ds(kk*4096, 4096), :], stg.at[u % NSTG].bitcast(bf16), ssems.at[u % NSTG])
    def x_piece(p, sem):
        return pltpu.make_async_copy(x_hbm.at[pl.ds(p*256, 256), :], xb.at[pl.ds(p*256, 256), :], wsems.at[sem])
    def wo_copy(n):
        return pltpu.make_async_copy(wo_hbm.at[:, pl.ds(n*128,128)], wo.at[n], wsems.at[0])
    xB_copy = pltpu.make_async_copy(x3_hbm.at[:, pl.ds(24, 8), :], xB3, wsems.at[3])
    def kvh_copies(j):
        cs = pl.ds(j*128, 128); sl = j % 2
        return [pltpu.make_async_copy(k_hbm.at[:, cs], kb.at[sl], sems.at[0, sl]),
                pltpu.make_async_copy(v_hbm.at[:, cs], vb.at[sl], sems.at[1, sl]),
                pltpu.make_async_copy(h_hbm.at[cs, :], hb.at[sl], sems.at[2, sl])]
    def q_copy(j):
        return pltpu.make_async_copy(q_hbm.at[:, pl.ds(j*128, 128)], qb.at[j % 2], sems.at[3, j % 2])
    ob_copy = pltpu.make_async_copy(ob, out_hbm.at[:, pl.ds(D, D)], osem.at[0])
    sgn = jnp.where(lax.broadcasted_iota(jnp.int32,(8,128),0) % 2 == 0, 1.0, -1.0).astype(f32)

    def fence():
        pl.semaphore_signal(fsem, 1)
        pl.semaphore_wait(fsem, 1)
    def s1_pre(j):
        l0 = j*128
        w = skT_ref[:, l0:l0+128].astype(f32)
        dd = d_ref[l0:l0+128].astype(f32).reshape(1, 128)
        return [jnp.broadcast_to(w[r:r+1], (8,128)) for r in range(4)], dd
    def s1_c(j, c, w, dd):
        Xh, Hh, kf = (X0, H0, kf0) if j % 2 == 0 else (X1, H1, kf1)
        sl = j % 2
        F = F_ref[...]
        kf[8+c*128:8+(c+1)*128, :] = kb[sl, c*128:(c+1)*128, :].astype(f32)
        kvs = []
        for r in range(16):
            b = 8 + c*128 + r*8
            kvs.append(kf[b:b+8, :]*w[0] + kf[b-1:b+7, :]*w[1] + kf[b-2:b+6, :]*w[2] + kf[b-3:b+5, :]*w[3])
        kv = (jnp.concatenate(kvs, axis=0) * vb[sl, c*128:(c+1)*128, :].astype(f32)).astype(bf16)
        xh = jnp.dot(F, kv, preferred_element_type=f32)
        hh = lax.dot_general(F, hb[sl, :, c*128:(c+1)*128], NT_, preferred_element_type=f32)
        e = hh[0:128]; f = hh[128:256]
        if c == 0: e = e + dd
        Xh[c, 0:256, :] = xh
        Hh[c, 0:128, :] = e
        if 0:
            Xh[c, 256:384, :] = xh[0:128] + xh[128:256]
            Hh[c, 128:256, :] = f - e
            Hh[c, 256:384, :] = e + f
        else:
            Hh[c, 128:256, :] = f
    BL = 4
    HK = []
    def s2_gen(j, g):
        Xh, Hh, Zb = (X0, H0, Z0) if j % 2 == 0 else (X1, H1, Z1)
        r0 = g*8; r1 = g*8+128; r2 = g*8+256
        M3 = 0
        def X(c): return (Xh[c, r0:r0+8, :], Xh[c, r1:r1+8, :], Xh[c, r2:r2+8, :]) if M3 else (Xh[c, r0:r0+8, :], Xh[c, r1:r1+8, :], None)
        def H(m): return (Hh[m, r0:r0+8, :], Hh[m, r1:r1+8, :], Hh[m, r2:r2+8, :]) if M3 else (Hh[m, r0:r0+8, :], Hh[m, r1:r1+8, :], None)
        prev = None
        for b in range(16//BL):
            acc = [None]*BL
            for m in range(BL*b+BL):
                he, hfe, hef = H(m)
                for i in range(BL):
                    c = BL*b+i
                    if m > c: continue
                    xa, xb_, xs_ = X(c-m)
                    p = (he*xs_, xa*hfe, xb_*hef) if M3 else (xa*he - xb_*hfe, xa*hfe + xb_*he)
                    acc[i] = p if acc[i] is None else tuple(a_+p_ for a_, p_ in zip(acc[i], p))
            for i in range(BL):
                c = BL*b+i
                yr, yi = (acc[i][0] - acc[i][2], acc[i][0] + acc[i][1]) if M3 else acc[i]
                if prev is None: zr, zi = yr, yi
                else: zr, zi = yr - sgn*prev[1], yi + sgn*prev[0]
                prev = (yr, yi)
                if 1:
                    zp = pltpu.bitcast(jnp.concatenate([zr, zi], axis=0).astype(bf16), u32)
                    Zb[c, r0:r0+8, :] = zp
                    HK.append(zp)
                else:
                    Zb[c, r0:r0+8, :] = zr; Zb[c, r1:r1+8, :] = zi
                    HK.append(pltpu.bitcast(zr, u32) | pltpu.bitcast(zi, u32))
            yield None
    def s3_c(j, c):
        Zb = Z0 if j % 2 == 0 else Z1
        G = G_ref[...]
        y = jnp.dot(G, bf(Zb[c]) if 1 else Zb[c].astype(bf16), preferred_element_type=f32)
        rs = slice(c*128,(c+1)*128)
        ob[rs, j*128:(j+1)*128] = (qb[j % 2, rs, :].astype(f32) * y).astype(bf16)

    def s1_q(j, cq, w, dd):
        Xh, Hh, kf = (X0, H0, kf0) if j % 2 == 0 else (X1, H1, kf1)
        sl = j % 2
        F = F_ref[...]
        kvl = []
        for c in range(4*cq, 4*cq+4):
            kf[8+c*128:8+(c+1)*128, :] = kb[sl, c*128:(c+1)*128, :].astype(f32)
            kvs = []
            for r in range(16):
                b = 8 + c*128 + r*8
                kvs.append(kf[b:b+8, :]*w[0] + kf[b-1:b+7, :]*w[1] + kf[b-2:b+6, :]*w[2] + kf[b-3:b+5, :]*w[3])
            kvl.append((jnp.concatenate(kvs, axis=0) * vb[sl, c*128:(c+1)*128, :].astype(f32)).astype(bf16))
        xh4 = jnp.dot(F, jnp.concatenate(kvl, axis=1), preferred_element_type=f32)
        hcat = jnp.concatenate([hb[sl, :, c*128:(c+1)*128] for c in range(4*cq, 4*cq+4)], axis=0)
        hh4 = lax.dot_general(F, hcat, NT_, preferred_element_type=f32)
        for i, c in enumerate(range(4*cq, 4*cq+4)):
            xh = xh4[:, i*128:(i+1)*128]; hh = hh4[:, i*128:(i+1)*128]
            e = hh[0:128]; f = hh[128:256]
            if c == 0: e = e + dd
            Xh[c, 0:256, :] = xh
            Hh[c, 0:128, :] = e
            if 0:
                Xh[c, 256:384, :] = xh[0:128] + xh[128:256]
                Hh[c, 128:256, :] = f - e
                Hh[c, 256:384, :] = e + f
            else:
                Hh[c, 128:256, :] = f
    def s3_q(j, cq):
        Zb = Z0 if j % 2 == 0 else Z1
        G = G_ref[...]
        z4 = jnp.concatenate([Zb[c] for c in range(4*cq, 4*cq+4)], axis=1)
        y4 = jnp.dot(G, bf(z4), preferred_element_type=f32)
        for i, c in enumerate(range(4*cq, 4*cq+4)):
            rs = slice(c*128,(c+1)*128)
            ob[rs, j*128:(j+1)*128] = (qb[j % 2, rs, :].astype(f32) * y4[:, i*128:(i+1)*128]).astype(bf16)
    def repack(u):
        mu, kk = u // 8, u % 8
        sl = u % NSTG
        for i in range(8):
            for j in range(16):
                Ev = stg[sl, pl.ds(256*i + j, 8, stride=32), :]
                Ov = stg[sl, pl.ds(256*i + 16 + j, 8, stride=32), :]
                r0 = kk*64 + 8*i
                wall[mu, r0:r0+8, 256*j:256*j+128] = (Ev & 0xffff) | (Ov << 16)
                wall[mu, r0:r0+8, 256*j+128:256*j+256] = (Ev >> 16) | (Ov & jnp.uint32(0xffff0000))
    def pm_kh(u, g):
        mu, kk = u // 8, u % 8
        pieces = [xB[8*r:8*r+8, 128*kk:128*kk+128] for r in range(32)]
        n = len(HK)
        if n:
            z = zr_ref[...]
            for i, hk in enumerate(HK):
                rg = 0 + (i * (32-0)) // n
                pieces[rg] = pieces[rg] | (hk & z)
            HK.clear()
        lhs = jnp.concatenate(pieces, axis=0)
        r = jnp.dot(bf(lhs), bf(wall[mu, kk*64:(kk+1)*64, g*512:(g+1)*512]), preferred_element_type=f32)
        if kk == 0: pre[mu, :, g*512:(g+1)*512] = r
        else: pre[mu, :, g*512:(g+1)*512] += r
    def pm_unit(u, gens):
        steps = [gi for gi in range(len(gens)) for _ in range(16 // BL)]
        n = len(steps)
        for g in range(8):
            for gi in steps[g*n//8:(g+1)*n//8]: next(gens[gi])
            pm_kh(u, g)
    def xb_prep():
        for i in range(NSEG//2):
            ab = jnp.concatenate([xB3[2*i], xB3[2*i+1]], axis=0)
            xB[8*i:8*i+8, :] = pltpu.bitcast(ab, u32)

    small = [pltpu.make_async_copy(a, b_, csem.at[i]) for i, (a, b_) in enumerate(
        ((zr_hbm, zr_ref), (F_hbm, F_ref), (skT_hbm, skT_ref), (d_hbm, d_ref), (G_hbm, G_ref), (mem_hbm, mem_ref)))]
    w_piece(0).start()
    xB_copy.start()
    for c in small: c.start()
    kf0[0:8, :] = jnp.zeros((8,128), f32); kf1[0:8, :] = jnp.zeros((8,128), f32)
    w_piece(0).wait()
    for c in kvh_copies(0): c.start()
    w_piece(1).start()
    for c in kvh_copies(1): c.start()
    w_piece(2).start()
    if 1 & 1: fence()
    with jax.named_scope('ph1'):
        repack(0)
        xB_copy.wait()
        xb_prep()
    QD = 0
    rng3 = (range(0,4), range(4,8), range(8,16)) if QD else (range(0,5), range(5,10), range(10,16))
    rng2 = (range(0,8), range(8,16))
    def sched(u):
        if u == 0: return None, False, []
        if u <= 21: return (u-1)//3, (u-1) % 3 == 0, rng3[(u-1) % 3]
        return 7, u == 22, rng2[u-22]
    with jax.named_scope('ph2'):
        for u in range(24):
            j, first, cs = sched(u)
            pm_unit(u, [s2_gen(j, c) for c in cs])
            if 0: fence()
            if u == 0:
                for c in small: c.wait()
                for c in kvh_copies(0): c.wait()
                w, dd = s1_pre(0)
                if QD:
                    for cq in range(4): s1_q(0, cq, w, dd)
                else:
                    for c in range(NC): s1_c(0, c, w, dd)
            else:
                if u == 1:
                    for c in kvh_copies(1): c.wait()
                if j + 1 < NT: w, dd = s1_pre(j+1)
                if QD:
                    for cq in range(cs[0]//4, (cs[-1]+1)//4):
                        if j + 1 < NT: s1_q(j+1, cq, w, dd)
                        if j >= 1: s3_q(j-1, cq)
                elif 0 == 0:
                    for c in cs:
                        if j + 1 < NT: s1_c(j+1, c, w, dd)
                        if j >= 1: s3_c(j-1, c)
                elif 0 == 1:
                    for c in cs:
                        if j + 1 < NT: s1_c(j+1, c, w, dd)
                    for c in cs:
                        if j >= 1: s3_c(j-1, c)
                else:
                    for c in cs:
                        if j >= 1: s3_c(j-1, c)
                    for c in cs:
                        if j + 1 < NT: s1_c(j+1, c, w, dd)
            if u < 23:
                w_piece(u+1).wait()
                jn, firstn, _ = sched(u+1)
                if firstn:
                    if jn + 1 < NT and jn > 0:
                        for c in kvh_copies(jn+1): c.wait()
                    if jn >= 1: q_copy(jn-1).wait()
                    if jn + 2 < NT:
                        for c in kvh_copies(jn+2): c.start()
                    q_copy(jn).start()
                if u + 3 < 24: w_piece(u+3).start()
                if 1 <= u < 17 and u % 2 == 1: wo_copy((u-1)//2).start()
                if u == 18: x_piece(0, 1).start()
                if 1 & 2: fence()
                repack(u+1)
        q_copy(NT-1).wait()
        if QD:
            for cq in range(4): s3_q(NT-1, cq)
        else:
            for c in range(NC): s3_c(NT-1, c)
        ob_copy.start()
    for n in range(8): wo_copy(n).wait()
    x_piece(0, 1).wait()
    for p in range(1, 8): x_piece(p, 2).start()

    membuf[...] = mem_ref[...].astype(f32)
    ri = lax.broadcasted_iota(jnp.int32, (40, 40), 0)
    ci = lax.broadcasted_iota(jnp.int32, (40, 40), 1)
    mask = (ri < 8) | (ri >= ci)
    c2 = float(128 ** -0.5 * np.log2(np.e))
    wou = wo.bitcast(u32)
    def step(s, mem):
        r0 = s * 32 if isinstance(s, int) else pl.multiple_of(s * 32, 32)
        p0 = s * 8 if isinstance(s, int) else pl.multiple_of(s * 8, 8)
        if 2 == 1:
            h = jnp.concatenate([mem.astype(bf16), xb[pl.ds(r0, 24), :]], axis=0)
        else:
            xs = xb[pl.ds(r0, 32), :].astype(f32)
            h = jnp.concatenate([mem, xs[0:24]], axis=0).astype(bf16)
        def proj(mu, g):
            cs = slice(g * 512, (g + 1) * 512)
            r = jnp.dot(h, bf(wall[mu, :, cs]), preferred_element_type=f32)
            return jnp.concatenate([r, pre[mu, pl.ds(p0, 8), cs]], axis=0)
        def scores(q, k):
            return [lax.dot_general(q[:, j*128:(j+1)*128], k[:, j*128:(j+1)*128], NT_, preferred_element_type=f32) for j in range(4)]
        def softmax(scs):
            ps = []
            for sc in scs:
                sc = jnp.where(mask, sc, -1e30)
                m = jnp.max(sc, axis=-1, keepdims=True)
                p = jnp.exp2((sc - m) * c2)
                l = jnp.sum(p, axis=-1, keepdims=True)
                r = pl.reciprocal(l, approx=True)
                r = r * (2.0 - l * r)
                ps.append(p * r)
            return ps
        def pv(ps, v, g):
            for j in range(4):
                o = jnp.dot(ps[j], v[:, j*128:(j+1)*128], preferred_element_type=f32)
                obuf[:, (g * 4 + j) * 128:(g * 4 + j + 1) * 128] = o
        def p1dots(ns):
            o1 = obuf[:, 0:3584]
            for n in ns:
                pbuf[:, n*128:(n+1)*128] = jnp.dot(o1, bf(wou[n, 0:1792, :]), preferred_element_type=f32)
        q = proj(0, 0); k = proj(1, 0); v = proj(2, 0)
        for g in range(8):
            if g + 1 < 8:
                qn = proj(0, g + 1)
                sc = scores(q, k)
                kn = proj(1, g + 1)
                ps = softmax(sc)
                vn = proj(2, g + 1)
                pv(ps, v, g)
                q, k, v = qn, kn, vn
            else:
                p1dots(range(2))
                sc = scores(q, k)
                p1dots(range(2, 5))
                ps = softmax(sc)
                pv(ps, v, g)
                p1dots(range(5, 8))
        o2 = obuf[:, 3584:4096]
        outs = [pbuf[:, n*128:(n+1)*128] + jnp.dot(o2, bf(wou[n, 1792:2048, :]), preferred_element_type=f32) for n in range(8)]
        outb = jnp.concatenate(outs, axis=1).astype(bf16)
        newmem = outb[0:8].astype(f32)
        aout[pl.ds(r0, 32), :] = outb[8:40]
        pltpu.make_async_copy(aout.at[pl.ds(r0, 32), :], out_hbm.at[pl.ds(r0, 32), pl.ds(0, D)], osem.at[1]).start()
        return newmem
    UN = 3
    PEEL = NSEG % UN
    def xwait():
        pltpu.make_async_copy(x_hbm.at[pl.ds(256, 7*256), :], xb.at[pl.ds(256, 7*256), :], wsems.at[2]).wait()
    def stepn(t, carry):
        @pl.when(t == (7 - PEEL) // UN)
        def _():
            xwait()
        mem = membuf[...]
        for u in range(UN):
            mem = step(PEEL + t*UN+u, mem)
        membuf[...] = mem
        return carry
    with jax.named_scope('chain'):
        if PEEL:
            mem = membuf[...]
            for s0 in range(PEEL): mem = step(s0, mem)
            membuf[...] = mem
        lax.fori_loop(0, NSEG//UN, stepn, 0)
    ob_copy.wait()
    pltpu.make_async_copy(aout, out_hbm.at[:, pl.ds(0, D)], osem.at[1]).wait()

@jax.jit
def pallas_concat_heads__memory_aug_recurrent_mem_tr__ssm_conv_h3__prompt_kernel(A_x, A_mem0, A_Wq, A_Wk, A_Wv, A_Wo, A_seg_len, B_q, B_k, B_v, B_shift_k, B_ssm_k, B_ssm_D):
    F,G = _consts()
    any_ = pl.BlockSpec(memory_space=pl.ANY)
    vm = pl.BlockSpec(memory_space=pltpu.VMEM)
    V = pltpu.VMEM
    out = pl.pallas_call(kernel, out_shape=jax.ShapeDtypeStruct((S,2*D), bf16),
        in_specs=[any_]*16, out_specs=any_,
        scratch_shapes=[V((8,128),u32), V((8,D),bf16), V((4,D),bf16), V((D,),bf16), V((256,128),bf16), V((128,256),bf16), pltpu.SemaphoreType.DMA((6,)), pltpu.SemaphoreType.REGULAR,
            V((S,D),bf16), V((64,8,D),bf16), V((256,D),u32), V((3,512,4096),u32),
            V((8,4096,128),bf16), V((NSTG,2048,128),u32), V((S,D),bf16), V((8,D),f32), V((40,4096),f32), V((40,1024),f32),
            V((3,512,4096),f32),
            V((2,S,128),bf16), V((2,S,128),bf16), V((2,S,128),bf16), V((2,128,S),bf16), V((S,D),bf16),
            V((NC,384,128),f32), V((NC,384,128),f32), V((NC,384,128),f32), V((NC,384,128),f32),
            *([V((NC,128,128),u32) if 1 else V((NC,256,128),f32)]*2), V((S+8,128),f32), V((S+8,128),f32),
            pltpu.SemaphoreType.DMA((4,2)), pltpu.SemaphoreType.DMA((4,)), pltpu.SemaphoreType.DMA((NSTG,)), pltpu.SemaphoreType.DMA((2,))],
        compiler_params=pltpu.CompilerParams(vmem_limit_bytes=124*1024*1024), name="kf",
    )(jnp.asarray(np.zeros((8,128), np.uint32)), A_x.reshape(S,D), A_x.reshape(64,32,D), A_mem0.reshape(8,D), A_Wq.reshape(32768,128), A_Wk.reshape(32768,128), A_Wv.reshape(32768,128),
      A_Wo.reshape(4096,D), B_q.reshape(S,D), B_k.reshape(S,D), B_v.reshape(S,D), B_shift_k.T, B_ssm_k, B_ssm_D,
      jnp.asarray(F).astype(bf16), jnp.asarray(G).astype(bf16))
    return out.reshape(1,S,2*D)
```

```python
import jax
import jax.numpy as jnp
import numpy as np
from jax import lax
from jax.experimental import pallas as pl
from jax.experimental.pallas import tpu as pltpu

S = 2048
D = 1024
NC = 16
NT = 8
NSEG = 64
UN = 3
NSTG = 4
BL = 4
bf16 = jnp.bfloat16
f32 = jnp.float32
u32 = jnp.uint32
NT_DIMS = (((1,), (1,)), ((), ()))


def _dft_matrices():
    k = np.arange(128)[:, None]
    t = np.arange(128)[None, :]
    th = np.pi * (2 * k + 1) * t / 256.0
    fwd = np.concatenate([np.cos(th), -np.sin(th)], axis=0)
    inv = np.concatenate([np.cos(th).T, -np.sin(th).T], axis=1) / 128.0
    perm = np.array([128 * p + 8 * g + r for g in range(16) for p in range(2) for r in range(8)])
    return fwd.astype(np.float32), inv[:, perm].astype(np.float32)


def _bf(x):
    return pltpu.bitcast(x, bf16)


def _kernel(zr_hbm, x_hbm, x3_hbm, mem_hbm, wq_hbm, wk_hbm, wv_hbm, wo_hbm,
            q_hbm, k_hbm, v_hbm, skT_hbm, h_hbm, d_hbm, F_hbm, G_hbm,
            out_hbm,
            zr_ref, mem_ref, skT_ref, d_ref, F_ref, G_ref, csem, fsem,
            xb, xB3, xB, wall, wo, stg, aout, membuf, obuf, pbuf, pre,
            kb, vb, qb, hb, ob, X0, H0, X1, H1, Z0, Z1, kf0, kf1,
            sems, wsems, ssems, osem):
    def w_piece(u):
        mu, kk = u // 8, u % 8
        src = (wq_hbm, wk_hbm, wv_hbm)[mu]
        return pltpu.make_async_copy(src.at[pl.ds(kk * 4096, 4096), :],
                                     stg.at[u % NSTG].bitcast(bf16), ssems.at[u % NSTG])

    def x_piece(p, sem):
        return pltpu.make_async_copy(x_hbm.at[pl.ds(p * 256, 256), :],
                                     xb.at[pl.ds(p * 256, 256), :], wsems.at[sem])

    def wo_copy(n):
        return pltpu.make_async_copy(wo_hbm.at[:, pl.ds(n * 128, 128)], wo.at[n], wsems.at[0])

    def kvh_copies(j):
        cs = pl.ds(j * 128, 128)
        sl = j % 2
        return [pltpu.make_async_copy(k_hbm.at[:, cs], kb.at[sl], sems.at[0, sl]),
                pltpu.make_async_copy(v_hbm.at[:, cs], vb.at[sl], sems.at[1, sl]),
                pltpu.make_async_copy(h_hbm.at[cs, :], hb.at[sl], sems.at[2, sl])]

    def q_copy(j):
        return pltpu.make_async_copy(q_hbm.at[:, pl.ds(j * 128, 128)], qb.at[j % 2], sems.at[3, j % 2])

    xB_copy = pltpu.make_async_copy(x3_hbm.at[:, pl.ds(24, 8), :], xB3, wsems.at[3])
    ob_copy = pltpu.make_async_copy(ob, out_hbm.at[:, pl.ds(D, D)], osem.at[0])
    small = [pltpu.make_async_copy(a, b_, csem.at[i]) for i, (a, b_) in enumerate(
        ((zr_hbm, zr_ref), (F_hbm, F_ref), (skT_hbm, skT_ref), (d_hbm, d_ref), (G_hbm, G_ref), (mem_hbm, mem_ref)))]
    sgn = jnp.where(lax.broadcasted_iota(jnp.int32, (8, 128), 0) % 2 == 0, 1.0, -1.0).astype(f32)

    def fence():
        pl.semaphore_signal(fsem, 1)
        pl.semaphore_wait(fsem, 1)

    def s1_pre(j):
        l0 = j * 128
        w = skT_ref[:, l0:l0 + 128].astype(f32)
        dd = d_ref[l0:l0 + 128].astype(f32).reshape(1, 128)
        return [jnp.broadcast_to(w[r:r + 1], (8, 128)) for r in range(4)], dd

    def s1_c(j, c, w, dd):
        Xh, Hh, kf = (X0, H0, kf0) if j % 2 == 0 else (X1, H1, kf1)
        sl = j % 2
        F = F_ref[...]
        kf[8 + c * 128:8 + (c + 1) * 128, :] = kb[sl, c * 128:(c + 1) * 128, :].astype(f32)
        kvs = []
        for r in range(16):
            b = 8 + c * 128 + r * 8
            kvs.append(kf[b:b + 8, :] * w[0] + kf[b - 1:b + 7, :] * w[1]
                       + kf[b - 2:b + 6, :] * w[2] + kf[b - 3:b + 5, :] * w[3])
        kv = (jnp.concatenate(kvs, axis=0) * vb[sl, c * 128:(c + 1) * 128, :].astype(f32)).astype(bf16)
        xh = jnp.dot(F, kv, preferred_element_type=f32)
        hh = lax.dot_general(F, hb[sl, :, c * 128:(c + 1) * 128], NT_DIMS, preferred_element_type=f32)
        e = hh[0:128]
        if c == 0:
            e = e + dd
        Xh[c, 0:256, :] = xh
        Hh[c, 0:128, :] = e
        Hh[c, 128:256, :] = hh[128:256]

    HK = []

    def s2_gen(j, g):
        Xh, Hh, Zb = (X0, H0, Z0) if j % 2 == 0 else (X1, H1, Z1)
        r0 = g * 8
        r1 = g * 8 + 128
        prev = None
        for b in range(NC // BL):
            acc = [None] * BL
            for m in range(BL * b + BL):
                he, hf = Hh[m, r0:r0 + 8, :], Hh[m, r1:r1 + 8, :]
                for i in range(BL):
                    c = BL * b + i
                    if m > c:
                        continue
                    xa, xi = Xh[c - m, r0:r0 + 8, :], Xh[c - m, r1:r1 + 8, :]
                    p = (xa * he - xi * hf, xa * hf + xi * he)
                    acc[i] = p if acc[i] is None else tuple(a_ + p_ for a_, p_ in zip(acc[i], p))
            for i in range(BL):
                c = BL * b + i
                yr, yi = acc[i]
                if prev is None:
                    zr, zi = yr, yi
                else:
                    zr, zi = yr - sgn * prev[1], yi + sgn * prev[0]
                prev = (yr, yi)
                zp = pltpu.bitcast(jnp.concatenate([zr, zi], axis=0).astype(bf16), u32)
                Zb[c, r0:r0 + 8, :] = zp
                HK.append(zp)
            yield None

    def s3_c(j, c):
        Zb = Z0 if j % 2 == 0 else Z1
        y = jnp.dot(G_ref[...], _bf(Zb[c]), preferred_element_type=f32)
        rs = slice(c * 128, (c + 1) * 128)
        ob[rs, j * 128:(j + 1) * 128] = (qb[j % 2, rs, :].astype(f32) * y).astype(bf16)

    def repack(u):
        mu, kk = u // 8, u % 8
        sl = u % NSTG
        for i in range(8):
            for j in range(16):
                ev = stg[sl, pl.ds(256 * i + j, 8, stride=32), :]
                od = stg[sl, pl.ds(256 * i + 16 + j, 8, stride=32), :]
                r0 = kk * 64 + 8 * i
                wall[mu, r0:r0 + 8, 256 * j:256 * j + 128] = (ev & 0xffff) | (od << 16)
                wall[mu, r0:r0 + 8, 256 * j + 128:256 * j + 256] = (ev >> 16) | (od & jnp.uint32(0xffff0000))

    def pm_kh(u, g):
        mu, kk = u // 8, u % 8
        pieces = [xB[8 * r:8 * r + 8, 128 * kk:128 * kk + 128] for r in range(32)]
        n = len(HK)
        if n:
            z = zr_ref[...]
            for i, hk in enumerate(HK):
                rg = (i * 32) // n
                pieces[rg] = pieces[rg] | (hk & z)
            HK.clear()
        lhs = jnp.concatenate(pieces, axis=0)
        r = jnp.dot(_bf(lhs), _bf(wall[mu, kk * 64:(kk + 1) * 64, g * 512:(g + 1) * 512]),
                    preferred_element_type=f32)
        if kk == 0:
            pre[mu, :, g * 512:(g + 1) * 512] = r
        else:
            pre[mu, :, g * 512:(g + 1) * 512] += r

    def pm_unit(u, gens):
        steps = [gi for gi in range(len(gens)) for _ in range(NC // BL)]
        n = len(steps)
        for g in range(8):
            for gi in steps[g * n // 8:(g + 1) * n // 8]:
                next(gens[gi])
            pm_kh(u, g)

    w_piece(0).start()
    xB_copy.start()
    for c in small:
        c.start()
    kf0[0:8, :] = jnp.zeros((8, 128), f32)
    kf1[0:8, :] = jnp.zeros((8, 128), f32)
    w_piece(0).wait()
    for c in kvh_copies(0):
        c.start()
    w_piece(1).start()
    for c in kvh_copies(1):
        c.start()
    w_piece(2).start()
    fence()
    repack(0)
    xB_copy.wait()
    for i in range(NSEG // 2):
        xB[8 * i:8 * i + 8, :] = pltpu.bitcast(jnp.concatenate([xB3[2 * i], xB3[2 * i + 1]], axis=0), u32)

    rng3 = (range(0, 5), range(5, 10), range(10, 16))
    rng2 = (range(0, 8), range(8, 16))

    def sched(u):
        if u == 0:
            return None, False, []
        if u <= 21:
            return (u - 1) // 3, (u - 1) % 3 == 0, rng3[(u - 1) % 3]
        return 7, u == 22, rng2[u - 22]

    for u in range(24):
        j, _, cs = sched(u)
        pm_unit(u, [s2_gen(j, c) for c in cs])
        if u == 0:
            for c in small:
                c.wait()
            for c in kvh_copies(0):
                c.wait()
            w, dd = s1_pre(0)
            for c in range(NC):
                s1_c(0, c, w, dd)
        else:
            if u == 1:
                for c in kvh_copies(1):
                    c.wait()
            if j + 1 < NT:
                w, dd = s1_pre(j + 1)
            for c in cs:
                if j + 1 < NT:
                    s1_c(j + 1, c, w, dd)
                if j >= 1:
                    s3_c(j - 1, c)
        if u < 23:
            w_piece(u + 1).wait()
            jn, firstn, _ = sched(u + 1)
            if firstn:
                if jn + 1 < NT and jn > 0:
                    for c in kvh_copies(jn + 1):
                        c.wait()
                if jn >= 1:
                    q_copy(jn - 1).wait()
                if jn + 2 < NT:
                    for c in kvh_copies(jn + 2):
                        c.start()
                q_copy(jn).start()
            if u + 3 < 24:
                w_piece(u + 3).start()
            if 1 <= u < 17 and u % 2 == 1:
                wo_copy((u - 1) // 2).start()
            if u == 18:
                x_piece(0, 1).start()
            repack(u + 1)
    q_copy(NT - 1).wait()
    for c in range(NC):
        s3_c(NT - 1, c)
    ob_copy.start()
    for n in range(8):
        wo_copy(n).wait()
    x_piece(0, 1).wait()
    for p in range(1, 8):
        x_piece(p, 2).start()

    membuf[...] = mem_ref[...].astype(f32)
    ri = lax.broadcasted_iota(jnp.int32, (40, 40), 0)
    ci = lax.broadcasted_iota(jnp.int32, (40, 40), 1)
    mask = (ri < 8) | (ri >= ci)
    c2 = float(128 ** -0.5 * np.log2(np.e))
    wou = wo.bitcast(u32)

    def step(s, mem):
        r0 = s * 32 if isinstance(s, int) else pl.multiple_of(s * 32, 32)
        p0 = s * 8 if isinstance(s, int) else pl.multiple_of(s * 8, 8)
        xs = xb[pl.ds(r0, 32), :].astype(f32)
        h = jnp.concatenate([mem, xs[0:24]], axis=0).astype(bf16)

        def proj(mu, g):
            cs = slice(g * 512, (g + 1) * 512)
            r = jnp.dot(h, _bf(wall[mu, :, cs]), preferred_element_type=f32)
            return jnp.concatenate([r, pre[mu, pl.ds(p0, 8), cs]], axis=0)

        def scores(q, k):
            return [lax.dot_general(q[:, j * 128:(j + 1) * 128], k[:, j * 128:(j + 1) * 128], NT_DIMS,
                                    preferred_element_type=f32) for j in range(4)]

        def softmax(scs):
            ps = []
            for sc in scs:
                sc = jnp.where(mask, sc, -1e30)
                m = jnp.max(sc, axis=-1, keepdims=True)
                p = jnp.exp2((sc - m) * c2)
                l = jnp.sum(p, axis=-1, keepdims=True)
                r = pl.reciprocal(l, approx=True)
                r = r * (2.0 - l * r)
                ps.append(p * r)
            return ps

        def pv(ps, v, g):
            for j in range(4):
                obuf[:, (g * 4 + j) * 128:(g * 4 + j + 1) * 128] = jnp.dot(
                    ps[j], v[:, j * 128:(j + 1) * 128], preferred_element_type=f32)

        def p1dots(ns):
            o1 = obuf[:, 0:3584]
            for n in ns:
                pbuf[:, n * 128:(n + 1) * 128] = jnp.dot(o1, _bf(wou[n, 0:1792, :]), preferred_element_type=f32)

        q = proj(0, 0)
        k = proj(1, 0)
        v = proj(2, 0)
        for g in range(8):
            if g + 1 < 8:
                qn = proj(0, g + 1)
                sc = scores(q, k)
                kn = proj(1, g + 1)
                ps = softmax(sc)
                vn = proj(2, g + 1)
                pv(ps, v, g)
                q, k, v = qn, kn, vn
            else:
                p1dots(range(2))
                sc = scores(q, k)
                p1dots(range(2, 5))
                ps = softmax(sc)
                pv(ps, v, g)
                p1dots(range(5, 8))
        o2 = obuf[:, 3584:4096]
        outs = [pbuf[:, n * 128:(n + 1) * 128]
                + jnp.dot(o2, _bf(wou[n, 1792:2048, :]), preferred_element_type=f32) for n in range(8)]
        outb = jnp.concatenate(outs, axis=1).astype(bf16)
        aout[pl.ds(r0, 32), :] = outb[8:40]
        pltpu.make_async_copy(aout.at[pl.ds(r0, 32), :], out_hbm.at[pl.ds(r0, 32), pl.ds(0, D)], osem.at[1]).start()
        return outb[0:8].astype(f32)

    PEEL = NSEG % UN

    def stepn(t, carry):
        @pl.when(t == (7 - PEEL) // UN)
        def _():
            pltpu.make_async_copy(x_hbm.at[pl.ds(256, 7 * 256), :], xb.at[pl.ds(256, 7 * 256), :], wsems.at[2]).wait()
        mem = membuf[...]
        for u in range(UN):
            mem = step(PEEL + t * UN + u, mem)
        membuf[...] = mem
        return carry

    mem = membuf[...]
    for s0 in range(PEEL):
        mem = step(s0, mem)
    membuf[...] = mem
    lax.fori_loop(0, NSEG // UN, stepn, 0)
    ob_copy.wait()
    pltpu.make_async_copy(aout, out_hbm.at[:, pl.ds(0, D)], osem.at[1]).wait()


@jax.jit
def pallas_concat_heads__memory_aug_recurrent_mem_tr__ssm_conv_h3__prompt_kernel(
    A_x, A_mem0, A_Wq, A_Wk, A_Wv, A_Wo, A_seg_len,
    B_q, B_k, B_v, B_shift_k, B_ssm_k, B_ssm_D,
):
    F, G = _dft_matrices()
    V = pltpu.VMEM
    DMA = pltpu.SemaphoreType.DMA
    out = pl.pallas_call(
        _kernel,
        out_shape=jax.ShapeDtypeStruct((S, 2 * D), bf16),
        in_specs=[pl.BlockSpec(memory_space=pl.ANY)] * 16,
        out_specs=pl.BlockSpec(memory_space=pl.ANY),
        scratch_shapes=[
            V((8, 128), u32), V((8, D), bf16), V((4, D), bf16), V((D,), bf16), V((256, 128), bf16), V((128, 256), bf16),
            DMA((6,)), pltpu.SemaphoreType.REGULAR,
            V((S, D), bf16), V((64, 8, D), bf16), V((256, D), u32), V((3, 512, 4096), u32),
            V((8, 4096, 128), bf16), V((NSTG, 2048, 128), u32), V((S, D), bf16), V((8, D), f32),
            V((40, 4096), f32), V((40, 1024), f32), V((3, 512, 4096), f32),
            V((2, S, 128), bf16), V((2, S, 128), bf16), V((2, S, 128), bf16), V((2, 128, S), bf16), V((S, D), bf16),
            V((NC, 256, 128), f32), V((NC, 256, 128), f32), V((NC, 256, 128), f32), V((NC, 256, 128), f32),
            V((NC, 128, 128), u32), V((NC, 128, 128), u32), V((S + 8, 128), f32), V((S + 8, 128), f32),
            DMA((4, 2)), DMA((4,)), DMA((NSTG,)), DMA((2,)),
        ],
        compiler_params=pltpu.CompilerParams(vmem_limit_bytes=124 * 1024 * 1024),
        name="kf",
    )(jnp.asarray(np.zeros((8, 128), np.uint32)),
      A_x.reshape(S, D), A_x.reshape(64, 32, D), A_mem0.reshape(8, D),
      A_Wq.reshape(32768, 128), A_Wk.reshape(32768, 128), A_Wv.reshape(32768, 128), A_Wo.reshape(4096, D),
      B_q.reshape(S, D), B_k.reshape(S, D), B_v.reshape(S, D), B_shift_k.T, B_ssm_k, B_ssm_D,
      jnp.asarray(F).astype(bf16), jnp.asarray(G).astype(bf16))
    return out.reshape(1, S, 2 * D)
```
